```python
import os as _os
_os.environ.setdefault("JAX_PLATFORMS", "cpu")
import jax
import jax.numpy as jnp

def _softmax(x, axis=-1):
    return jax.nn.softmax(x, axis=axis)
def _gelu(x):
    return jax.nn.gelu(x, approximate=True)
def _silu(x):
    return jax.nn.silu(x)
def _sigmoid(x):
    return jax.nn.sigmoid(x)
def _layernorm(x, axis=-1, eps=1e-5):
    m = jnp.mean(x, axis=axis, keepdims=True)
    v = jnp.var(x, axis=axis, keepdims=True)
    return (x - m) / jnp.sqrt(v + eps)
def _scatter_add(tgt, idx, src, axis=0):
    return tgt.at[idx].add(src)
def _segment_sum(src, seg, n):
    return jax.ops.segment_sum(src, seg, n)
class _Rng:
    def __init__(self, key):
        self._k = key
    def _next(self):
        self._k, sub = jax.random.split(self._k)
        return sub
    def normal(self, shape):
        return jax.random.normal(self._next(), shape, dtype=jnp.bfloat16)
    def randint(self, lo, hi, shape):
        return jax.random.randint(self._next(), shape, lo, hi, dtype=jnp.int32)
    def uniform(self, shape, lo=0.0, hi=1.0):
        return jax.random.uniform(self._next(), shape, jnp.bfloat16, lo, hi)
    def permutation(self, n):
        return jax.random.permutation(self._next(), n)


kernel_name = 'sequential_preLN__mha_block__dense_activation_squared_relu__prompt'

def setup_inputs():
    _rng = _Rng(jax.random.key(int.from_bytes(__import__("os").urandom(4), "little")))
    _w = (lambda a: (lambda t: t.astype(jnp.bfloat16) if jnp.issubdtype(t.dtype, jnp.floating) else t)(jnp.asarray(a)))
    def _A_setup():
        B, S, D, H = 1, 2048, 448, 16
        return {
            "x": _w((lambda *s: _rng.normal(s) * 0.05)(B, S, D)),
            "wqkv": _w((lambda *s: _rng.normal(s) * 0.05)(D, 3 * D)),
            "wo": _w((lambda *s: _rng.normal(s) * 0.05)(D, D)),
        }
    _A_in = _A_setup()

    def _B_setup():
        B, S, D, F = 1, 2048, 448, 1792
        return {
            "x": _w((lambda *s: _rng.normal(s) * 0.05)(B, S, D)),
            "w1": _w((lambda *s: _rng.normal(s) * 0.05)(D, F)),
            "b1": _w((lambda *s: _rng.normal(s) * 0.05)(F)),
            "w2": _w((lambda *s: _rng.normal(s) * 0.05)(F, D)),
            "b2": _w((lambda *s: _rng.normal(s) * 0.05)(D)),
        }
    _B_in = _B_setup()

    return {
        "A_x": _A_in["x"],
        "A_wqkv": _A_in["wqkv"],
        "A_wo": _A_in["wo"],
        "B_x": _B_in["x"],
        "B_w1": _B_in["w1"],
        "B_b1": _B_in["b1"],
        "B_w2": _B_in["w2"],
        "B_b2": _B_in["b2"],
    }

def reference(A_x, A_wqkv, A_wo, B_x, B_w1, B_b1, B_w2, B_b2):
    def _A_ref(x, wqkv, wo):
        B, S, D = x.shape
        H = 16
        Dh = D // H
        qkv = (lambda x, *d: x.transpose(*d))((x @ wqkv).reshape(B, S, 3, H, Dh), 2, 0, 3, 1, 4)
        q, k, v = qkv[0], qkv[1], qkv[2]
        scores = jnp.einsum("bhqd,bhkd->bhqk", q, k) * (Dh ** -0.5)
        p = _softmax(scores, axis=-1)
        o = jnp.einsum("bhqk,bhkd->bhqd", p, v)
        return (lambda x, *d: x.transpose(*d))(o, 0, 2, 1, 3).reshape(B, S, D) @ wo

    def _B_ref(x, w1, b1, w2, b2):
        h = jnp.einsum("bsd,df->bsf", x, w1) + b1
        zero = jnp.zeros_like(h)
        r = jnp.where(h > zero, h, zero)
        h = r * r
        out = jnp.einsum("bsf,fd->bsd", h, w2) + b2
        return out

    x = A_x
    h = x + _A_ref(_layernorm(x, axis=-1), A_wqkv, A_wo)
    h2 = h + _B_ref(_layernorm(h, axis=-1), B_w1, B_b1, B_w2, B_b2)
    return h2
```

```python
import functools
import math

import jax
import jax.numpy as jnp
from jax import lax
import jax.experimental.pallas as pl
import jax.experimental.pallas.tpu as pltpu

BF = jnp.bfloat16
F32 = jnp.float32
U32 = jnp.uint32

H = 16
DH = 28
HP = 32
GH = 4
GW = GH * DH
EPS = 1e-5
DP = 512


def _pk(x):
    return pltpu.bitcast(x, U32)


def _upk(x):
    return pltpu.bitcast(x, BF)


def _layernorm_t(x):
    m = jnp.mean(x, axis=0, keepdims=True)
    xc = x - m
    v = jnp.mean(xc * xc, axis=0, keepdims=True)
    return xc * lax.rsqrt(v + EPS)


def _kernel(xt_hbm, wqkv_hbm, wo_hbm, w1_hbm, b1_ref, w2t_hbm, b2_ref, out_ref,
            xt_v, wqkv_v, wo_v, w1_v, w2t_v, sems,
            wt_s, wot_s, w1t_s, b2_s, wtmp_s, k_s, qt_s, vt_s, ot_s,
            s0, s1, m0, m1, p0, p1, q0, q1, *, S, D, F, TQ, U, TA, TC, SKIP=""):
    NQB = S // TQ
    NI = NQB * H
    NB = NI // U
    NA = S // TA
    step = pl.program_id(0)
    qscale = (DH ** -0.5) * math.log2(math.e)

    def x_copy(b):
        return pltpu.make_async_copy(xt_hbm.at[:, pl.ds(b * TA, TA)], xt_v.at[b], sems.at[b])

    wqkv_copy = pltpu.make_async_copy(wqkv_hbm, wqkv_v, sems.at[NA])
    wo_copy = pltpu.make_async_copy(wo_hbm, wo_v, sems.at[NA + 1])
    w1_copy = pltpu.make_async_copy(w1_hbm, w1_v, sems.at[NA + 2])
    w2_copy = pltpu.make_async_copy(w2t_hbm, w2t_v, sems.at[NA + 3])

    @pl.when(step == 0)
    def _phase_ab():
        wqkv_copy.start()
        for b in range(NA):
            x_copy(b).start()
        wo_copy.start()
        w1_copy.start()
        w2_copy.start()

        wqkv_copy.wait()
        wt_s[pl.ds(0, D), :] = _pk(wqkv_v[:, pl.ds(0, 2 * D)].astype(F32).T.astype(BF))
        wtmp_s[...] = wqkv_v[:, pl.ds(3 * D - 512, 512)].astype(F32).T
        zero4 = jnp.zeros((HP - DH, D), F32)
        for h in range(H):
            blk = jnp.concatenate([wtmp_s[pl.ds(512 - D + DH * h, DH), :], zero4], axis=0)
            wt_s[pl.ds(D + HP * h // 2, HP // 2), :] = _pk(blk.astype(BF))

        vrow = lax.broadcasted_iota(jnp.int32, (H * HP, TA), 0)
        is_one = (vrow % HP) == DH
        for b in range(NA):
            x_copy(b).wait()
            cols = pl.ds(b * TA, TA)
            xn = _layernorm_t(xt_v[b].astype(F32)).astype(BF)
            qkv = jnp.dot(_upk(wt_s[...]), xn, preferred_element_type=F32)
            qb, qo = (b * TA) // TQ, (b * TA) % TQ
            qt_s[qb, :, pl.ds(qo, TA)] = qkv[:D + 16] * qscale
            for g in range(H // GH):
                kt = qkv[D + GW * g:D + GW * g + 128]
                k_s[g, pl.ds(b * TA // 2, TA // 2), :] = _pk(kt.T.astype(BF))
            vt_s[:, cols] = _pk(jnp.where(is_one, 1.0, qkv[2 * D:]).astype(BF))

        row = lax.broadcasted_iota(jnp.int32, (128, TQ), 0)

        def stage0(t, q_ref):
            t = jnp.minimum(t, NI - 1)
            qb = t // H
            h = t % H
            g = h // GH
            lo = DH * (h % GH)
            q = qt_s[qb, pl.ds(pl.multiple_of(GW * g, 16), 128), :]
            q_ref[...] = _pk(jnp.where((row >= lo) & (row < lo + DH), q, 0.0).astype(BF))

        def stage1(t, q_ref, s_ref, m_ref):
            g = (t % H) // GH
            s = jnp.dot(_upk(k_s[g]), _upk(q_ref[...]), preferred_element_type=F32)
            s_ref[...] = s
            m_ref[...] = jnp.max(s.reshape(S // 8, 8, TQ), axis=0)

        def stage2(s_ref, m_ref, p_ref):
            m = jnp.max(m_ref[...], axis=0, keepdims=True)
            kc = 16
            for c in range(S // kc):
                p_ref[pl.ds(c * kc // 2, kc // 2), :] = _pk(
                    jnp.exp2(s_ref[pl.ds(c * kc, kc), :] - m).astype(BF))

        def stage3(t, p_ref):
            qb = t // H
            h = t % H
            v = _upk(vt_s[pl.ds(pl.multiple_of(HP // 2 * h, HP // 2), HP // 2), :])
            o = jnp.dot(v, _upk(p_ref[...]), preferred_element_type=F32)
            ot_s[qb, pl.ds(pl.multiple_of(HP * h, HP), HP), :] = o

        def prep_c():
            wo_copy.wait()
            wtmp_s[pl.ds(0, D), :] = wo_v[...].astype(F32)
            blks = []
            for h in range(H):
                blks += [wtmp_s[pl.ds(DH * h, DH), :], zero4]
            wot_s[...] = _pk(jnp.concatenate(blks, axis=0).T.astype(BF))
            w1_copy.wait()
            rr = lax.broadcasted_iota(jnp.int32, (DP - D, F), 0)
            tail = jnp.where(rr == 0, b1_ref[...].astype(F32), 0.0)
            w1a = jnp.concatenate([w1_v[...].astype(F32), tail], axis=0)
            w1t_s[...] = _pk(w1a.T.astype(BF))
            b2_s[...] = jnp.broadcast_to(b2_ref[...].astype(F32), (128, D)).T
            w2_copy.wait()

        for u in range(U):
            stage0(u, q0.at[u])
        for u in range(U):
            stage0(U + u, q1.at[u])
        for u in range(U):
            stage1(u, q0.at[u], s0.at[u], m0.at[u])
        prep_c()
        for u in range(U):
            stage0(2 * U + u, q0.at[u])
        for u in range(U):
            stage1(U + u, q1.at[u], s1.at[u], m1.at[u])
            stage2(s0.at[u], m0.at[u], p0.at[u])

        def half(b, sa, ma, sb, mb, pb, pa, qa, qb_):
            for u in range(U):
                stage1((b + 2) * U + u, qa.at[u], sa.at[u], ma.at[u])
                stage2(sb.at[u], mb.at[u], pb.at[u])
                stage0((b + 3) * U + u, qb_.at[u])
                stage3(b * U + u, pa.at[u])

        def body(t, c):
            @pl.when(t % 2 == 0)
            def _():
                half(t, s0, m0, s1, m1, p1, p0, q0, q1)

            @pl.when(t % 2 == 1)
            def _():
                half(t, s1, m1, s0, m0, p0, p1, q1, q0)
            return c

        lax.fori_loop(0, 2 if "B" in SKIP else NB - 2, body, 0)
        for u in range(U):
            stage2(s1.at[u], m1.at[u], p1.at[u])
            stage3((NB - 2) * U + u, p0.at[u])
        for u in range(U):
            stage3((NB - 1) * U + u, p1.at[u])

    assert TQ == TC and TA == TC
    ot = ot_s[step].reshape(H, HP, TC)
    ot = (ot * (1.0 / ot[:, DH:DH + 1, :])).reshape(H * HP, TC).astype(BF)
    hh = xt_v[step].astype(F32) + jnp.dot(_upk(wot_s[...]), ot, preferred_element_type=F32)
    if "C" in SKIP:
        out_ref[...] = hh.astype(out_ref.dtype)
        return
    rr = lax.broadcasted_iota(jnp.int32, (DP - D, TC), 0)
    hn = jnp.concatenate([_layernorm_t(hh), jnp.where(rr == 0, 1.0, 0.0)], axis=0).astype(BF)
    a = jnp.dot(_upk(w1t_s[...]), hn, preferred_element_type=F32)
    a = jnp.maximum(a, 0.0)
    a = (a * a).astype(BF)
    y = jnp.dot(w2t_v[...], a, preferred_element_type=F32)
    b2 = jnp.concatenate([b2_s[...]] * (TC // 128), axis=1)
    out_ref[...] = (hh + y + b2).astype(out_ref.dtype)


def _build(A_x, A_wqkv, A_wo, B_x, B_w1, B_b1, B_w2, B_b2, TQ=512, U=2, TA=512, TC=512, SKIP=""):
    B, S, D = A_x.shape
    F = B_w1.shape[1]
    assert B == 1 and D == H * DH
    NQB = S // TQ
    NA = S // TA
    xt = jnp.swapaxes(A_x, 1, 2).reshape(D, S)
    full = lambda shape: pl.BlockSpec(shape, lambda i: (0,) * len(shape))
    hbm = pl.BlockSpec(memory_space=pltpu.MemorySpace.HBM)
    out = pl.pallas_call(
        functools.partial(_kernel, S=S, D=D, F=F, TQ=TQ, U=U, TA=TA, TC=TC, SKIP=SKIP),
        grid=(S // TC,),
        in_specs=[hbm, hbm, hbm, hbm, full((1, F)), hbm, full((1, D))],
        out_specs=pl.BlockSpec((D, TC), lambda i: (0, i)),
        out_shape=jax.ShapeDtypeStruct((D, S), A_x.dtype),
        scratch_shapes=[
            pltpu.VMEM((NA, D, TA), BF),
            pltpu.VMEM((D, 3 * D), BF),
            pltpu.VMEM((D, D), BF),
            pltpu.VMEM((D, F), BF),
            pltpu.VMEM((D, F), BF),
            pltpu.SemaphoreType.DMA((NA + 4,)),
            pltpu.VMEM(((2 * D + H * HP) // 2, D), U32),
            pltpu.VMEM((D // 2, H * HP), U32),
            pltpu.VMEM((F // 2, DP), U32),
            pltpu.VMEM((D, 128), F32),
            pltpu.VMEM((512, D), F32),
            pltpu.VMEM((H // GH, S // 2, 128), U32),
            pltpu.VMEM((NQB, D + 16, TQ), F32),
            pltpu.VMEM((H * HP // 2, S), U32),
            pltpu.VMEM((NQB, H * HP, TQ), F32),
            pltpu.VMEM((U, S, TQ), F32), pltpu.VMEM((U, S, TQ), F32),
            pltpu.VMEM((U, 8, TQ), F32), pltpu.VMEM((U, 8, TQ), F32),
            pltpu.VMEM((U, S // 2, TQ), U32), pltpu.VMEM((U, S // 2, TQ), U32),
            pltpu.VMEM((U, 64, TQ), U32), pltpu.VMEM((U, 64, TQ), U32),
        ],
        compiler_params=pltpu.CompilerParams(
            dimension_semantics=("arbitrary",),
            vmem_limit_bytes=100 * 1024 * 1024),
    )(xt, A_wqkv, A_wo, B_w1, B_b1.reshape(1, F), B_w2.T, B_b2.reshape(1, D))
    return jnp.swapaxes(out.reshape(B, D, S), 1, 2)


@jax.jit
def pallas_sequential_preLN__mha_block__dense_activation_squared_relu__prompt_kernel(
    A_x: jax.Array,
    A_wqkv: jax.Array,
    A_wo: jax.Array,
    B_x: jax.Array,
    B_w1: jax.Array,
    B_b1: jax.Array,
    B_w2: jax.Array,
    B_b2: jax.Array,
):
    return _build(A_x, A_wqkv, A_wo, B_x, B_w1, B_b1, B_w2, B_b2)
```

```python
import functools
import math

import jax
import jax.numpy as jnp
from jax import lax
import jax.experimental.pallas as pl
import jax.experimental.pallas.tpu as pltpu

BF = jnp.bfloat16
F32 = jnp.float32
U32 = jnp.uint32

H = 16
DH = 28
HP = 32
GH = 4
NG = H // GH
GW = GH * DH
EPS = 1e-5
DP = 512
CR = 16


def _pk(x):
    return pltpu.bitcast(x, U32)


def _upk(x):
    return pltpu.bitcast(x, BF)


def _dot(a, b):
    return jnp.dot(a, b, preferred_element_type=F32)


def _rows(start, size, align):
    if isinstance(start, int):
        return pl.ds(start, size)
    return pl.ds(pl.multiple_of(start, align), size)


def _colsum(x, chains=1):
    if chains == 1:
        return jnp.sum(x, axis=0, keepdims=True)
    rows = [x[r:r + 8] for r in range(0, x.shape[0], 8)]
    parts = [functools.reduce(jnp.add, rows[c::chains]) for c in range(chains)]
    return jnp.sum(functools.reduce(jnp.add, parts), axis=0, keepdims=True)


def _shifted_moments(x, chains=1):
    inv_n = 1.0 / x.shape[0]
    d = x - x[0:1]
    dm = _colsum(d, chains) * inv_n
    var = jnp.maximum(_colsum(d * d, chains) * inv_n - dm * dm, 0.0)
    return d, dm, var


def _layernorm_t(x):
    inv_n = 1.0 / x.shape[0]
    xc = x - _colsum(x) * inv_n
    return xc * lax.rsqrt(_colsum(xc * xc) * inv_n + EPS)


def _strassen_lhs(a11, a12, a21, a22):
    return (a11 + a22, a21 + a22, a11, a22, a11 + a12, a21 - a11, a12 - a22)


def _strassen_rhs(b11, b12, b21, b22):
    return (b11 + b22, b11, b12 - b22, b21 - b11, b22, b11 + b12, b21 + b22)


def _strassen(lhs_ref, rhs, cr, tmp, sink):
    u0, u1, u2 = tmp
    for k in (4, 2, 1, 3, 0, 6, 5):
        mk = _dot(_upk(lhs_ref.at[k][...]), rhs[k])
        for r in range(0, mk.shape[0], cr):
            rows = pl.ds(r, cr)
            z = mk[r:r + cr]
            if k == 4:
                u1[rows, :] = z
            elif k == 2:
                sink(0, 1, r, u1[rows, :] + z)
                u0[rows, :] = z
            elif k == 1:
                u0[rows, :] = u0[rows, :] - z
                u2[rows, :] = z
            elif k == 3:
                sink(1, 0, r, u2[rows, :] + z)
                u1[rows, :] = z - u1[rows, :]
            elif k == 0:
                u2[rows, :] = z
            elif k == 6:
                sink(0, 0, r, u2[rows, :] + u1[rows, :] + z)
            else:
                sink(1, 1, r, u2[rows, :] + u0[rows, :] + z)


def _kernel(xt_hbm, wqkv_hbm, wo_hbm, w1_hbm, b1_hbm, w2t_hbm, b2_hbm, out_hbm,
            xt_v, wqkv_v, wo_v, w1_v, w2t_v, out_v, sems, osem,
            wt_s, aqk_s, av_s, wot_s, a1_s, a2_s, b2_s, wtmp_s, k_s, qt_s, vt_s, ot_s, h_s, st_s,
            s_s, p_s, m_s, o_s, b1_v, b2_v, *, S, D, F, T):
    NQ = S // T
    NT = T // 128
    NGI = NQ * NG
    TH, KH = T // 2, DP // 2
    qscale = (DH ** -0.5) * math.log2(math.e)

    def x_copy(b):
        return pltpu.make_async_copy(xt_hbm.at[:, pl.ds(b * T, T)], xt_v.at[b], sems.at[b])

    def w_copy(lo, hi, i):
        return pltpu.make_async_copy(wqkv_hbm.at[:, pl.ds(lo, hi - lo)],
                                     wqkv_v.at[:, pl.ds(lo, hi - lo)], sems.at[NQ + i])

    wa_copy, wb_copy = w_copy(384, 640, 0), w_copy(640, 2 * D, 1)
    wc_copy, wv_copy = w_copy(0, 384, 2), w_copy(2 * D, 3 * D, 3)
    wo_copy = pltpu.make_async_copy(wo_hbm, wo_v, sems.at[NQ + 4])
    w1_copy = pltpu.make_async_copy(w1_hbm, w1_v, sems.at[NQ + 5])
    w2_copy = pltpu.make_async_copy(w2t_hbm, w2t_v, sems.at[NQ + 6])
    b1_copy = pltpu.make_async_copy(b1_hbm, b1_v, sems.at[NQ + 7])
    b2_copy = pltpu.make_async_copy(b2_hbm, b2_v, sems.at[NQ + 8])

    for c in (wa_copy, x_copy(0), wb_copy, wc_copy, wv_copy, x_copy(1), x_copy(2), x_copy(3),
              wo_copy, w1_copy, b1_copy, b2_copy, w2_copy):
        c.start()

    def x_tile(b, n):
        return xt_v.at[b][:, pl.ds(128 * n, 128)].astype(F32)

    def store_q(b, row, col, q):
        qt_s[pl.ds((b * D + row) // 2, q.shape[0] // 2), pl.ds(col, q.shape[1])] = _pk(
            (q * qscale).astype(BF))

    def store_k(g, tok, kt):
        kt = jnp.concatenate([kt, jnp.zeros((128 - GW, kt.shape[1]), F32)], axis=0)
        k_s[pl.ds((g * S + tok) // 2, kt.shape[1] // 2), :] = _pk(kt.T.astype(BF))

    def wt_chunk(lo, n=128):
        wt = wqkv_v[:, pl.ds(lo, n)].astype(F32).T.astype(BF)
        wt_s[pl.ds(lo // 2, n // 2), :] = _pk(wt)
        return wt

    wa_copy.wait()
    wt3 = wt_chunk(384)
    wt4 = wt_chunk(512)
    x_copy(0).wait()
    xn0 = []
    for n in range(NT):
        d, dm, var = _shifted_moments(x_tile(0, n), 2)
        xn0.append(((d - dm) * lax.rsqrt(var + EPS)).astype(BF))
    xn0 = jnp.concatenate(xn0, axis=1)
    ra = _dot(jnp.concatenate([wt3, wt4], axis=0), xn0[:, :TH])
    rb = _dot(wt3, xn0[:, TH:])
    wb_copy.wait()
    wc_copy.wait()
    rc = _dot(wt4, xn0[:, TH:])
    r34 = jnp.concatenate([ra, jnp.concatenate([rb, rc], axis=0)], axis=1)
    store_q(0, 384, 0, r34[:D - 384])
    k0 = jnp.concatenate([r34[D - 384:]] + [_dot(wt_chunk(lo), xn0) for lo in (640, 768)], axis=0)
    for g in range(NG):
        store_k(g, 0, k0[GW * g:GW * (g + 1)])
    for lo in (0, 128):
        store_q(0, lo, 0, _dot(wt_chunk(lo), xn0))
    wt2 = wt_chunk(256)

    wv_copy.wait()
    x_copy(1).wait()
    store_q(0, 256, 0, _dot(wt2, xn0))
    vt_s[pl.ds(D // 2, 8), :] = jnp.zeros((8, S), U32)

    def prep_lhs(dst, top, bot, n):
        zl = jnp.zeros((CR, DP - D), F32)
        for r in range(0, n, CR):
            t = _upk(wt_s[pl.ds((top + r) // 2, CR // 2), :]).astype(F32)
            b = _upk(wt_s[pl.ds((bot + r) // 2, CR // 2), :]).astype(F32)
            ops = _strassen_lhs(t[:, :KH], jnp.concatenate([t[:, KH:], zl], axis=1),
                                b[:, :KH], jnp.concatenate([b[:, KH:], zl], axis=1))
            for k in range(7):
                dst.at[k][pl.ds(r // 2, CR // 2), :] = _pk(ops[k].astype(BF))

    prep_lhs(aqk_s, 0, D, D)
    wt_chunk(2 * D, D)
    prep_lhs(av_s, 2 * D, 2 * D + D // 2, D // 2)

    def rhs_ops(xn):
        zr = jnp.zeros((DP - D, TH), F32)
        ops = _strassen_rhs(xn[:KH, :TH], xn[:KH, TH:],
                            jnp.concatenate([xn[KH:, :TH], zr], axis=0),
                            jnp.concatenate([xn[KH:, TH:], zr], axis=0))
        return [op.astype(BF) for op in ops]

    def ln1_ops(b):
        return rhs_ops(jnp.concatenate([_layernorm_t(x_tile(b, n)) for n in range(NT)], axis=1))

    def tmp(slot, n):
        return [s_s.at[slot, pl.ds(k * D, n), pl.ds(0, TH)] for k in range(3)]

    def qk_block(b, rhs):
        def sink(r, c, row, z):
            if r == 0:
                store_q(b, row, c * TH, z)
            else:
                store_k(row // GW, b * T + c * TH, z)
        _strassen(aqk_s, rhs, GW, tmp(b % 2, D), sink)

    def v_block(b, rhs):
        def sink(r, c, row, z):
            vt_s[pl.ds((r * D // 2 + row) // 2, CR // 2), pl.ds(b * T + c * TH, TH)] = _pk(
                z.astype(BF))
        _strassen(av_s, rhs, CR, tmp(2 + b % 2, D // 2), sink)

    rhs1 = ln1_ops(1)
    qk_block(1, rhs1)
    v_block(0, rhs_ops(xn0.astype(F32)))
    for c in (x_copy(2), x_copy(3), wo_copy, w1_copy, b1_copy):
        c.wait()
    v_block(1, rhs1)
    for b in range(2, NQ):
        rhs = ln1_ops(b)
        qk_block(b, rhs)
        v_block(b, rhs)

    prow = lax.broadcasted_iota(jnp.int32, (GW // 2, T), 0)
    qzero = jnp.zeros((64 - GW // 2, T), U32)
    vrow = lax.broadcasted_iota(jnp.int32, (HP // 2, S), 0)
    vtail = _pk(jnp.where(lax.broadcasted_iota(jnp.int32, (HP, S), 0) == DH, 1.0, 0.0).astype(BF))

    def scores(gi, j):
        lo = DH // 2 * j
        q = qt_s[_rows(GW // 2 * gi, GW // 2, 8), :]
        q = jnp.where((prow >= lo) & (prow < lo + DH // 2), q, jnp.uint32(0))
        q = jnp.concatenate([q, qzero], axis=0)
        s = _dot(_upk(k_s[_rows((gi & (NG - 1)) * (S // 2), S // 2, S // 2), :]), _upk(q))
        s_s.at[j][...] = s
        m_s.at[j][...] = jnp.max(s.reshape(S // 8, 8, T), axis=0)

    def probs(j, lo=0, hi=S // CR):
        m = jnp.max(m_s.at[j][...], axis=0, keepdims=True)
        for c in range(lo, hi):
            p_s.at[j][pl.ds(c * CR // 2, CR // 2), :] = _pk(
                jnp.exp2(s_s.at[j][pl.ds(c * CR, CR), :] - m).astype(BF))

    def pv(gi, j):
        lo = DH // 2 * j
        al = lo // 8 * 8
        v = vt_s[_rows((gi & (NG - 1)) * (GW // 2) + al, 24, 8), :][lo - al:lo - al + HP // 2]
        v = jnp.where(vrow < DH // 2, v, vtail)
        o_s.at[j][...] = _dot(_upk(v), _upk(p_s.at[j][...]))

    def normalize(gi, j):
        off = gi * (GH * HP // 2) + j * (HP // 2)
        o = o_s.at[j][...]
        o = o * (1.0 / o[DH:DH + 1, :])
        ot_s[_rows(off, HP // 2, HP // 2), :] = _pk(o.astype(BF))

    def prep_wo_w1():
        wtmp_s[pl.ds(0, D // 2), :] = _pk(wo_v[...])
        wtmp_s[pl.ds(D // 2, 8), :] = jnp.zeros((8, D), U32)
        r = lax.broadcasted_iota(jnp.int32, (HP // 2, D), 0)
        wop = jnp.concatenate(
            [jnp.where(r < DH // 2, wtmp_s[pl.ds(DH // 2 * h, HP // 2), :], jnp.uint32(0))
             for h in range(H)], axis=0)
        wot_s[...] = _pk(_upk(wop).astype(F32).T.astype(BF))
        rr = lax.broadcasted_iota(jnp.int32, (DP - D, 128), 0)
        b1 = b1_v[...].astype(F32).reshape(1, F)

        def w1t(r):
            tail = jnp.where(rr == 0, b1[:, 128 * r:128 * (r + 1)], 0.0)
            return jnp.concatenate([w1_v[:, pl.ds(128 * r, 128)].astype(F32), tail], axis=0).T

        for r in range(F // 256):
            t1, t2 = w1t(r), w1t(r + F // 256)
            ops = _strassen_lhs(t1[:, :KH], t1[:, KH:], t2[:, :KH], t2[:, KH:])
            for k in range(7):
                a1_s.at[k][pl.ds(64 * r, 64), :] = _pk(ops[k].astype(BF))

    def prep_w2(c):
        top = w2t_v[_rows(16 * c, 16, 16), :].astype(F32)
        bot = w2t_v[_rows(D // 2 + 16 * c, 16, 16), :].astype(F32)
        ops = _strassen_lhs(top[:, :F // 2], top[:, F // 2:], bot[:, :F // 2], bot[:, F // 2:])
        for k in range(7):
            a2_s.at[k][_rows(8 * c, 8, 8), :] = _pk(ops[k].astype(BF))

    def out_proj(t):
        i, n = t // NT, t % NT
        ot = _upk(ot_s[pl.ds(i * H * HP // 2, H * HP // 2), pl.ds(128 * n, 128)])
        hh = x_tile(i, n) + _dot(_upk(wot_s[...]), ot)
        h_s.at[t][...] = hh
        _, dm, var = _shifted_moments(hh)
        st_s.at[t][pl.ds(0, 8), :] = jnp.broadcast_to(hh[0:1] + dm, (8, 128))
        st_s.at[t][pl.ds(8, 8), :] = jnp.broadcast_to(var, (8, 128))

    def rstd(t):
        st_s.at[t][pl.ds(8, 8), :] = lax.rsqrt(st_s.at[t][pl.ds(8, 8), :] + EPS)

    o_s[...] = jnp.ones(o_s.shape, F32)
    for j in range(GH):
        scores(0, j)
        if j == 0:
            prep_wo_w1()
    w2_copy.wait()

    def body(gi, carry):
        for j in range(GH):
            normalize(jnp.maximum(gi - 1, 0), j)
            probs(j)
            scores(gi + 1, j)
            if j == 1:
                prep_w2(jnp.minimum(gi, D // 32 - 1))
            pv(gi, j)
        return carry

    lax.fori_loop(0, NGI - 1, body, 0)

    gl = NGI - 1
    nfirst = (NQ - 1) * NT - 2
    nch = S // CR
    for j in range(GH):
        normalize(gl - 1, j)
    for t in range(nfirst):
        lo, hi = t * GH * nch // nfirst, (t + 1) * GH * nch // nfirst
        while lo < hi:
            j = lo // nch
            e = min(hi, (j + 1) * nch)
            probs(j, lo - j * nch, e - j * nch)
            lo = e
        out_proj(t)
    b2_copy.wait()
    b2_s[...] = jnp.broadcast_to(b2_v[...].astype(F32).reshape(1, D), (128, D)).T
    for j in range(GH):
        pv(gl, j)
        normalize(gl, j)
    for t in range(nfirst):
        rstd(t)
    for t in range(nfirst, NQ * NT):
        out_proj(t)
        rstd(t)

    def out_copy(i, r, c):
        return pltpu.make_async_copy(
            out_v.at[i * 4 + r * 2 + c],
            out_hbm.at[pl.ds(r * D // 2, D // 2), _rows(i * T + c * TH, TH, TH)], osem)

    tmps = [s_s.at[k // 2, pl.ds(0, F // 2), pl.ds(k % 2 * TH, TH)] for k in range(6)]
    ab = [p_s.at[k // 2, pl.ds(0, F // 4), pl.ds(k % 2 * TH, TH)] for k in range(7)]
    htail = jnp.where(lax.broadcasted_iota(jnp.int32, (DP - D, TH), 0) == 0, 1.0, 0.0)

    def ffn(i, carry):
        def hn(r, c):
            lo, hi = r * KH, min((r + 1) * KH, D)
            cols = []
            for n in range(NT // 2):
                t = i * NT + c * NT // 2 + n
                z = h_s.at[t][pl.ds(lo, hi - lo), :].reshape((hi - lo) // 8, 8, 128)
                z = (z - st_s.at[t][pl.ds(0, 8), :]) * st_s.at[t][pl.ds(8, 8), :]
                cols.append(z.reshape(hi - lo, 128))
            z = jnp.concatenate(cols, axis=1)
            return z if r == 0 else jnp.concatenate([z, htail], axis=0)

        a11, a12, a21 = tmps[3:]

        def sink(r, c, row, z):
            rows = pl.ds(row, CR)
            a = jnp.square(jnp.maximum(z, 0.0))

            def put(k, val):
                ab[k][pl.ds(row // 2, CR // 2), :] = _pk(val.astype(BF))

            if (r, c) == (0, 1):
                a12[rows, :] = a
            elif (r, c) == (1, 0):
                a21[rows, :] = a
            elif (r, c) == (0, 0):
                a11[rows, :] = a
                put(1, a)
                put(3, a21[rows, :] - a)
                put(5, a + a12[rows, :])
            else:
                put(0, a11[rows, :] + a)
                put(2, a12[rows, :] - a)
                put(4, a)
                put(6, a21[rows, :] + a)

        rhs = [op.astype(BF) for op in _strassen_rhs(hn(0, 0), hn(0, 1), hn(1, 0), hn(1, 1))]
        _strassen(a1_s, rhs, CR, tmps[:3], sink)

        def emit(r, c, y):
            rows = pl.ds(r * D // 2, D // 2)
            hh = jnp.concatenate(
                [h_s.at[i * NT + c * NT // 2 + n][rows, :] + b2_s[rows, :] for n in range(NT // 2)],
                axis=1)
            out_v.at[i * 4 + r * 2 + c][...] = (hh + y).astype(BF)
            out_copy(i, r, c).start()

        m = {}
        for k in (1, 3, 5, 0, 2, 4, 6):
            m[k] = _dot(_upk(a2_s.at[k][...]), _upk(ab[k][...]))
            if k == 3:
                emit(1, 0, m[1] + m[3])
            if k == 2:
                emit(1, 1, m[0] - m[1] + m[2] + m[5])
            if k == 4:
                emit(0, 1, m[2] + m[4])
            if k == 6:
                emit(0, 0, m[0] + m[3] - m[4] + m[6])
        return carry

    lax.fori_loop(0, NQ, ffn, 0)
    for i in range(NQ):
        for r in range(2):
            for c in range(2):
                out_copy(i, r, c).wait()


@jax.jit
def pallas_sequential_preLN__mha_block__dense_activation_squared_relu__prompt_kernel(
    A_x: jax.Array,
    A_wqkv: jax.Array,
    A_wo: jax.Array,
    B_x: jax.Array,
    B_w1: jax.Array,
    B_b1: jax.Array,
    B_w2: jax.Array,
    B_b2: jax.Array,
):
    B, S, D = A_x.shape
    F = B_w1.shape[1]
    T = 512
    NQ = S // T
    assert B == 1 and D == H * DH and NQ == 4 and F % 256 == 0
    xt = jnp.swapaxes(A_x, 1, 2).reshape(D, S)
    hbm = pl.BlockSpec(memory_space=pltpu.MemorySpace.HBM)
    out = pl.pallas_call(
        functools.partial(_kernel, S=S, D=D, F=F, T=T),
        in_specs=[hbm] * 7,
        out_specs=hbm,
        out_shape=jax.ShapeDtypeStruct((D, S), A_x.dtype),
        scratch_shapes=[
            pltpu.VMEM((NQ, D, T), BF),
            pltpu.VMEM((D, 3 * D), BF),
            pltpu.VMEM((D, D), BF),
            pltpu.VMEM((D, F), BF),
            pltpu.VMEM((D, F), BF),
            pltpu.VMEM((NQ * 4, D // 2, T // 2), BF),
            pltpu.SemaphoreType.DMA((NQ + 9,)),
            pltpu.SemaphoreType.DMA(()),
            pltpu.VMEM((3 * D // 2, D), U32),
            pltpu.VMEM((7, D // 2, DP // 2), U32),
            pltpu.VMEM((7, D // 4, DP // 2), U32),
            pltpu.VMEM((D // 2, H * HP), U32),
            pltpu.VMEM((7, F // 4, DP // 2), U32),
            pltpu.VMEM((8, D // 4, F // 2), U32),
            pltpu.VMEM((D, 128), F32),
            pltpu.VMEM((D // 2 + 8, D), U32),
            pltpu.VMEM((NG * S // 2, 128), U32),
            pltpu.VMEM((NQ * D // 2, T), U32),
            pltpu.VMEM((D // 2 + 8, S), U32),
            pltpu.VMEM((NQ * H * HP // 2, T), U32),
            pltpu.VMEM((S // 128, D, 128), F32),
            pltpu.VMEM((S // 128, 16, 128), F32),
            pltpu.VMEM((GH, S, T), F32),
            pltpu.VMEM((GH, S // 2, T), U32),
            pltpu.VMEM((GH, 8, T), F32),
            pltpu.VMEM((GH, HP, T), F32),
            pltpu.VMEM((F,), BF),
            pltpu.VMEM((D,), BF),
        ],
        compiler_params=pltpu.CompilerParams(vmem_limit_bytes=100 * 1024 * 1024,
                                             disable_bounds_checks=True,
                                             disable_semaphore_checks=True),
    )(xt, A_wqkv, A_wo, B_w1, B_b1, B_w2.T, B_b2)
    return jnp.swapaxes(out.reshape(B, D, S), 1, 2)
```

```python
import functools
import math

import jax
import jax.numpy as jnp
from jax import lax
import jax.experimental.pallas as pl
import jax.experimental.pallas.tpu as pltpu

BF = jnp.bfloat16
F32 = jnp.float32
U32 = jnp.uint32

H = 16
DH = 28
HP = 32
GH = 4
NG = H // GH
GW = GH * DH
EPS = 1e-5
DP = 512
CR = 16
VPU_KEYS = (112, 144, 144, 128)
VPU_LATE = (4, 4, 4, 3)


def _pk(x):
    return pltpu.bitcast(x, U32)


def _upk(x):
    return pltpu.bitcast(x, BF)


def _dot(a, b):
    return jnp.dot(a, b, preferred_element_type=F32)


def _after(x, dep):
    zero = (pltpu.bitcast(dep, U32) >> 31) >> 1
    return pltpu.bitcast(pltpu.bitcast(x, U32) | zero, x.dtype)


def _rows(start, size, align):
    if isinstance(start, int):
        return pl.ds(start, size)
    return pl.ds(pl.multiple_of(start, align), size)


def _colsum(x, chains=1):
    if chains == 1:
        return jnp.sum(x, axis=0, keepdims=True)
    rows = [x[r:r + 8] for r in range(0, x.shape[0], 8)]
    parts = [functools.reduce(jnp.add, rows[c::chains]) for c in range(chains)]
    return jnp.sum(functools.reduce(jnp.add, parts), axis=0, keepdims=True)


def _shifted_moments(x, chains=1):
    inv_n = 1.0 / x.shape[0]
    d = x - x[0:1]
    dm = _colsum(d, chains) * inv_n
    var = jnp.maximum(_colsum(d * d, chains) * inv_n - dm * dm, 0.0)
    return d, dm, var


def _layernorm_t(x):
    inv_n = 1.0 / x.shape[0]
    xc = x - _colsum(x) * inv_n
    return xc * lax.rsqrt(_colsum(xc * xc) * inv_n + EPS)


def _strassen_lhs(a11, a12, a21, a22):
    return (a11 + a22, a21 + a22, a11, a22, a11 + a12, a21 - a11, a12 - a22)


def _strassen_rhs(b11, b12, b21, b22):
    return (b11 + b22, b11, b12 - b22, b21 - b11, b22, b11 + b12, b21 + b22)


def _strassen(lhs_ref, rhs, cr, tmp, sink):
    u0, u1, u2 = tmp
    for k in (4, 2, 1, 3, 0, 6, 5):
        mk = _dot(_upk(lhs_ref.at[k][...]), rhs[k])
        for r in range(0, mk.shape[0], cr):
            rows = pl.ds(r, cr)
            z = mk[r:r + cr]
            if k == 4:
                u1[rows, :] = z
            elif k == 2:
                sink(0, 1, r, u1[rows, :] + z)
                u0[rows, :] = z
            elif k == 1:
                u0[rows, :] = u0[rows, :] - z
                u2[rows, :] = z
            elif k == 3:
                sink(1, 0, r, u2[rows, :] + z)
                u1[rows, :] = z - u1[rows, :]
            elif k == 0:
                u2[rows, :] = z
            elif k == 6:
                sink(0, 0, r, u2[rows, :] + u1[rows, :] + z)
            else:
                sink(1, 1, r, u2[rows, :] + u0[rows, :] + z)


def _kernel(xt_hbm, wqkv_hbm, wo_hbm, w1_hbm, b1_hbm, w2t_hbm, b2_hbm, out_hbm,
            xt_v, wqkv_v, wo_v, w1_v, w2t_v, out_v, sems, osem,
            wt_s, aqk_s, av_s, wot_s, a1_s, a2_s, b2_s, wtmp_s, k_s, qt_s, vp_s, ot_s, h_s, st_s,
            qb_s, kf_s, s_s, p_s, m_s, o_s, b1_v, b2_v, *, S, D, F, T):
    NQ = S // T
    NT = T // 128
    NGI = NQ * NG
    TH, KH = T // 2, DP // 2
    qscale = (DH ** -0.5) * math.log2(math.e)

    def x_copy(b):
        return pltpu.make_async_copy(xt_hbm.at[:, pl.ds(b * T, T)], xt_v.at[b], sems.at[b])

    def w_copy(lo, hi, i):
        return pltpu.make_async_copy(wqkv_hbm.at[:, pl.ds(lo, hi - lo)],
                                     wqkv_v.at[:, pl.ds(lo, hi - lo)], sems.at[NQ + i])

    wa_copy, wb_copy = w_copy(384, 640, 0), w_copy(640, 2 * D, 1)
    wc_copy, wv_copy = w_copy(0, 384, 2), w_copy(2 * D, 3 * D, 3)
    wo_copy = pltpu.make_async_copy(wo_hbm, wo_v, sems.at[NQ + 4])
    w1_copy = pltpu.make_async_copy(w1_hbm, w1_v, sems.at[NQ + 5])
    w2_copy = pltpu.make_async_copy(w2t_hbm, w2t_v, sems.at[NQ + 6])
    b1_copy = pltpu.make_async_copy(b1_hbm, b1_v, sems.at[NQ + 7])
    b2_copy = pltpu.make_async_copy(b2_hbm, b2_v, sems.at[NQ + 8])

    for c in (wa_copy, x_copy(0), wb_copy, wc_copy, wv_copy, x_copy(1), x_copy(2), x_copy(3),
              wo_copy, w1_copy, b1_copy, b2_copy, w2_copy):
        c.start()

    def x_tile(b, n):
        return xt_v.at[b][:, pl.ds(128 * n, 128)].astype(F32)

    def store_q(b, row, col, q):
        qt_s[pl.ds((b * D + row) // 2, q.shape[0] // 2), pl.ds(col, q.shape[1])] = _pk(
            (q * qscale).astype(BF))

    def store_k(g, tok, kt):
        kt = jnp.concatenate([kt, jnp.zeros((128 - GW, kt.shape[1]), F32)], axis=0)
        k = kt.T.astype(BF)
        k_s[pl.ds((g * S + tok) // 2, kt.shape[1] // 2), :] = _pk(k)
        if tok == 0:
            kf_s.at[g][...] = k[:160].astype(F32)

    def wt_chunk(lo, n=128):
        wt = wqkv_v[:, pl.ds(lo, n)].astype(F32).T.astype(BF)
        wt_s[pl.ds(lo // 2, n // 2), :] = _pk(wt)
        return wt

    def prep_lhs(dst, top, bot, n):
        zl = jnp.zeros((CR, DP - D), F32)
        for r in range(0, n, CR):
            t = _upk(wt_s[pl.ds((top + r) // 2, CR // 2), :]).astype(F32)
            b = _upk(wt_s[pl.ds((bot + r) // 2, CR // 2), :]).astype(F32)
            ops = _strassen_lhs(t[:, :KH], jnp.concatenate([t[:, KH:], zl], axis=1),
                                b[:, :KH], jnp.concatenate([b[:, KH:], zl], axis=1))
            for k in range(7):
                dst.at[k][pl.ds(r // 2, CR // 2), :] = _pk(ops[k].astype(BF))

    wa_copy.wait()
    wt3 = wt_chunk(384)
    wt4 = wt_chunk(512)
    x_copy(0).wait()
    xn0 = []
    for n in range(NT):
        d, dm, var = _shifted_moments(x_tile(0, n), 2)
        xn0.append(((d - dm) * lax.rsqrt(var + EPS)).astype(BF))
    xn0 = jnp.concatenate(xn0, axis=1)
    ra = _dot(jnp.concatenate([wt3, wt4], axis=0), xn0[:, :TH])
    rb = _dot(wt3, xn0[:, TH:])
    wb_copy.wait()
    wc_copy.wait()
    rc = _dot(wt4, xn0[:, TH:])
    r34 = jnp.concatenate([ra, jnp.concatenate([rb, rc], axis=0)], axis=1)
    store_q(0, 384, 0, r34[:D - 384])
    k0 = jnp.concatenate([r34[D - 384:]] + [_dot(wt_chunk(lo), xn0) for lo in (640, 768)], axis=0)
    for g in range(NG):
        store_k(g, 0, k0[GW * g:GW * (g + 1)])
    for lo in (0, 128):
        store_q(0, lo, 0, _dot(wt_chunk(lo), xn0))
    wt2 = wt_chunk(256)

    wv_copy.wait()
    x_copy(1).wait()
    store_q(0, 256, 0, _dot(wt2, xn0))

    prep_lhs(aqk_s, 0, D, D)
    wt_chunk(2 * D, D)
    prep_lhs(av_s, 2 * D, 2 * D + D // 2, D // 2)

    def rhs_ops(xn):
        zr = jnp.zeros((DP - D, TH), F32)
        ops = _strassen_rhs(xn[:KH, :TH], xn[:KH, TH:],
                            jnp.concatenate([xn[KH:, :TH], zr], axis=0),
                            jnp.concatenate([xn[KH:, TH:], zr], axis=0))
        return [op.astype(BF) for op in ops]

    def ln1_ops(b):
        return rhs_ops(jnp.concatenate([_layernorm_t(x_tile(b, n)) for n in range(NT)], axis=1))

    def tmp(slot, n):
        return [s_s.at[slot, pl.ds(k * D, n), pl.ds(0, TH)] for k in range(3)]

    def qk_block(b, rhs):
        def sink(r, c, row, z):
            if r == 0:
                store_q(b, row, c * TH, z)
            else:
                store_k(row // GW, b * T + c * TH, z)
        _strassen(aqk_s, rhs, GW, tmp(b % 2, D), sink)

    vtail = jnp.where(lax.broadcasted_iota(jnp.int32, (HP - DH, TH), 0) == 0, 1.0, 0.0)

    def v_block(b, rhs):
        def sink(r, c, row, z):
            for jj in range(2):
                h = (r * D // 2 + row) // DH + jj
                v = jnp.concatenate([z[DH * jj:DH * (jj + 1)], vtail], axis=0)
                vp_s[pl.ds(HP // 2 * h, HP // 2), pl.ds(b * T + c * TH, TH)] = _pk(v.astype(BF))
        _strassen(av_s, rhs, 2 * DH, tmp(2 + b % 2, D // 2), sink)

    rhs1 = ln1_ops(1)
    qk_block(1, rhs1)
    v_block(0, rhs_ops(xn0.astype(F32)))
    for c in (x_copy(2), x_copy(3), wo_copy, w1_copy, b1_copy):
        c.wait()
    v_block(1, rhs1)
    for b in range(2, NQ):
        rhs = ln1_ops(b)
        qk_block(b, rhs)
        v_block(b, rhs)

    prow = lax.broadcasted_iota(jnp.int32, (GW // 2, T), 0)
    qzero = jnp.zeros((64 - GW // 2, T), U32)

    def scores_mxu(gi, j, first):
        lo = DH // 2 * j
        q = qt_s[_rows(GW // 2 * gi, GW // 2, 8), :]
        q = jnp.where((prow >= lo) & (prow < lo + DH // 2), q, jnp.uint32(0))
        q = jnp.concatenate([q, qzero], axis=0)
        k = k_s[_rows((gi & (NG - 1)) * (S // 2) + first // 2, (S - first) // 2, 8), :]
        s = _dot(_upk(k), _upk(q))
        s_s.at[j][pl.ds(first, S - first), :] = s
        return s

    def scores_vpu(gi, j, r, mx, dep=None):
        kr = kf_s.at[gi & (NG - 1)][pl.ds(r, 8), :]
        acc = [None] * NT
        for d in range(DH):
            kb = jnp.broadcast_to(kr[:, DH * j + d:DH * j + d + 1], (8, 128))
            for n in range(NT):
                z = kb * qb_s.at[j][pl.ds(8 * (d * NT + n), 8), :]
                acc[n] = z if acc[n] is None else acc[n] + z
        for n in range(NT):
            z = acc[n] if dep is None else _after(acc[n], dep)
            s_s.at[j][pl.ds(r, 8), pl.ds(128 * n, 128)] = z
            mx[n] = z if mx[n] is None else jnp.maximum(mx[n], z)

    def scores(gi, j):
        s = scores_mxu(gi, j, VPU_KEYS[j])
        nr = s.shape[0] // 8
        early = VPU_KEYS[j] // 8 - VPU_LATE[j]
        skip = 40 if j == 0 else 0
        mx = [None] * NT
        done = 0
        for i in range(nr):
            for n in range(NT):
                z = s[8 * i:8 * i + 8, 128 * n:128 * (n + 1)]
                mx[n] = z if mx[n] is None else jnp.maximum(mx[n], z)
            while done < min(early, int((i + 1 - skip) * early / (nr * 0.92 - skip))):
                scores_vpu(gi, j, 8 * done, mx)
                done += 1
        assert done == early
        m_s.at[j][pl.ds(0, 8), :] = jnp.concatenate(mx, axis=1)

    def scores_late(gi, j, o):
        mx = [None] * NT
        for u in range(VPU_LATE[j]):
            r = VPU_KEYS[j] - 8 * (VPU_LATE[j] - u)
            scores_vpu(gi, j, r, mx, o[:8, 128 * u:128 * (u + 1)])
        m_s.at[j][pl.ds(8, 8), :] = jnp.concatenate(mx, axis=1)

    def spread_q(gi, j, pace=None):
        lo = DH * j // 16 * 16
        q = _upk(qt_s[_rows(GW // 2 * gi + lo // 2, 24 if j < GH - 1 else 16, 8), :]).astype(F32)
        for d in range(DH):
            r = DH * j + d - lo
            for n in range(NT):
                z = jnp.broadcast_to(q[r:r + 1, 128 * n:128 * (n + 1)], (8, 128))
                if pace is not None:
                    z = _after(z, pace[64 * d:64 * d + 8, :128])
                qb_s.at[j][pl.ds(8 * (d * NT + n), 8), :] = z

    def probs(j, lo=0, hi=S // CR):
        m = jnp.max(m_s.at[j][...], axis=0, keepdims=True)
        for c in range(lo, hi):
            p_s.at[j][pl.ds(c * CR // 2, CR // 2), :] = _pk(
                jnp.exp2(s_s.at[j][pl.ds(c * CR, CR), :] - m).astype(BF))

    def pv(gi, j):
        off = (gi & (NG - 1)) * (GH * HP // 2) + j * (HP // 2)
        o = _dot(_upk(vp_s[_rows(off, HP // 2, HP // 2), :]), _upk(p_s.at[j][...]))
        o_s.at[j][...] = o
        return o

    def normalize(gi, j):
        off = gi * (GH * HP // 2) + j * (HP // 2)
        o = o_s.at[j][...]
        o = o * (1.0 / o[DH:DH + 1, :])
        ot_s[_rows(off, HP // 2, HP // 2), :] = _pk(o.astype(BF))

    def prep_wo_w1():
        wtmp_s[pl.ds(0, D // 2), :] = _pk(wo_v[...])
        wtmp_s[pl.ds(D // 2, 8), :] = jnp.zeros((8, D), U32)
        r = lax.broadcasted_iota(jnp.int32, (HP // 2, D), 0)
        wop = jnp.concatenate(
            [jnp.where(r < DH // 2, wtmp_s[pl.ds(DH // 2 * h, HP // 2), :], jnp.uint32(0))
             for h in range(H)], axis=0)
        wot_s[...] = _pk(_upk(wop).astype(F32).T.astype(BF))
        rr = lax.broadcasted_iota(jnp.int32, (DP - D, 128), 0)
        b1 = b1_v[...].astype(F32).reshape(1, F)

        def w1t(r):
            tail = jnp.where(rr == 0, b1[:, 128 * r:128 * (r + 1)], 0.0)
            return jnp.concatenate([w1_v[:, pl.ds(128 * r, 128)].astype(F32), tail], axis=0).T

        for r in range(F // 256):
            t1, t2 = w1t(r), w1t(r + F // 256)
            ops = _strassen_lhs(t1[:, :KH], t1[:, KH:], t2[:, :KH], t2[:, KH:])
            for k in range(7):
                a1_s.at[k][pl.ds(64 * r, 64), :] = _pk(ops[k].astype(BF))

    def prep_w2(c):
        top = w2t_v[_rows(16 * c, 16, 16), :].astype(F32)
        bot = w2t_v[_rows(D // 2 + 16 * c, 16, 16), :].astype(F32)
        ops = _strassen_lhs(top[:, :F // 2], top[:, F // 2:], bot[:, :F // 2], bot[:, F // 2:])
        for k in range(7):
            a2_s.at[k][_rows(8 * c, 8, 8), :] = _pk(ops[k].astype(BF))

    def out_proj(t):
        i, n = t // NT, t % NT
        ot = _upk(ot_s[pl.ds(i * H * HP // 2, H * HP // 2), pl.ds(128 * n, 128)])
        hh = x_tile(i, n) + _dot(_upk(wot_s[...]), ot)
        h_s.at[t][...] = hh
        _, dm, var = _shifted_moments(hh)
        st_s.at[t][pl.ds(0, 8), :] = jnp.broadcast_to(hh[0:1] + dm, (8, 128))
        st_s.at[t][pl.ds(8, 8), :] = jnp.broadcast_to(var, (8, 128))

    def rstd(t):
        st_s.at[t][pl.ds(8, 8), :] = lax.rsqrt(st_s.at[t][pl.ds(8, 8), :] + EPS)

    o_s[...] = jnp.ones(o_s.shape, F32)
    for j in range(GH):
        s = scores_mxu(0, j, 0)
        m_s.at[j][...] = jnp.max(s.reshape(S // 16, 16, T), axis=0)
        spread_q(1, j, s)
        if j == 0:
            prep_wo_w1()
    w2_copy.wait()

    def body(gi, carry):
        for j in range(GH):
            normalize(jnp.maximum(gi - 1, 0), j)
            probs(j)
            scores(gi + 1, j)
            scores_late(gi + 1, j, pv(gi, j))
            spread_q(jnp.minimum(gi + 2, NGI - 1), j)
        prep_w2(jnp.minimum(gi, D // 32 - 1))
        return carry

    lax.fori_loop(0, NGI - 1, body, 0)

    gl = NGI - 1
    nfirst = (NQ - 1) * NT - 2
    nch = S // CR
    for j in range(GH):
        normalize(gl - 1, j)
    for t in range(nfirst):
        lo, hi = t * GH * nch // nfirst, (t + 1) * GH * nch // nfirst
        while lo < hi:
            j = lo // nch
            e = min(hi, (j + 1) * nch)
            probs(j, lo - j * nch, e - j * nch)
            lo = e
        out_proj(t)
    b2_copy.wait()
    b2_s[...] = jnp.broadcast_to(b2_v[...].astype(F32).reshape(1, D), (128, D)).T
    for j in range(GH):
        pv(gl, j)
        normalize(gl, j)
    for t in range(nfirst):
        rstd(t)
    for t in range(nfirst, NQ * NT):
        out_proj(t)
        rstd(t)

    def out_copy(i, r, c):
        return pltpu.make_async_copy(
            out_v.at[i * 4 + r * 2 + c],
            out_hbm.at[pl.ds(r * D // 2, D // 2), _rows(i * T + c * TH, TH, TH)], osem)

    tmps = [s_s.at[k // 2, pl.ds(0, F // 2), pl.ds(k % 2 * TH, TH)] for k in range(6)]
    ab = [p_s.at[k // 2, pl.ds(0, F // 4), pl.ds(k % 2 * TH, TH)] for k in range(7)]
    htail = jnp.where(lax.broadcasted_iota(jnp.int32, (DP - D, TH), 0) == 0, 1.0, 0.0)

    def ffn(i, carry):
        def hn(r, c):
            lo, hi = r * KH, min((r + 1) * KH, D)
            cols = []
            for n in range(NT // 2):
                t = i * NT + c * NT // 2 + n
                z = h_s.at[t][pl.ds(lo, hi - lo), :].reshape((hi - lo) // 8, 8, 128)
                z = (z - st_s.at[t][pl.ds(0, 8), :]) * st_s.at[t][pl.ds(8, 8), :]
                cols.append(z.reshape(hi - lo, 128))
            z = jnp.concatenate(cols, axis=1)
            return z if r == 0 else jnp.concatenate([z, htail], axis=0)

        a11, a12, a21 = tmps[3:]

        def sink(r, c, row, z):
            rows = pl.ds(row, CR)
            a = jnp.square(jnp.maximum(z, 0.0))

            def put(k, val):
                ab[k][pl.ds(row // 2, CR // 2), :] = _pk(val.astype(BF))

            if (r, c) == (0, 1):
                a12[rows, :] = a
            elif (r, c) == (1, 0):
                a21[rows, :] = a
            elif (r, c) == (0, 0):
                a11[rows, :] = a
                put(1, a)
                put(3, a21[rows, :] - a)
                put(5, a + a12[rows, :])
            else:
                put(0, a11[rows, :] + a)
                put(2, a12[rows, :] - a)
                put(4, a)
                put(6, a21[rows, :] + a)

        rhs = [op.astype(BF) for op in _strassen_rhs(hn(0, 0), hn(0, 1), hn(1, 0), hn(1, 1))]
        _strassen(a1_s, rhs, CR, tmps[:3], sink)

        def emit(r, c, y):
            rows = pl.ds(r * D // 2, D // 2)
            hh = jnp.concatenate(
                [h_s.at[i * NT + c * NT // 2 + n][rows, :] + b2_s[rows, :] for n in range(NT // 2)],
                axis=1)
            out_v.at[i * 4 + r * 2 + c][...] = (hh + y).astype(BF)
            out_copy(i, r, c).start()

        m = {}
        for k in (1, 3, 5, 0, 2, 4, 6):
            m[k] = _dot(_upk(a2_s.at[k][...]), _upk(ab[k][...]))
            if k == 3:
                emit(1, 0, m[1] + m[3])
            if k == 2:
                emit(1, 1, m[0] - m[1] + m[2] + m[5])
            if k == 4:
                emit(0, 1, m[2] + m[4])
            if k == 6:
                emit(0, 0, m[0] + m[3] - m[4] + m[6])
        return carry

    lax.fori_loop(0, NQ, ffn, 0)
    for i in range(NQ):
        for r in range(2):
            for c in range(2):
                out_copy(i, r, c).wait()


@jax.jit
def pallas_sequential_preLN__mha_block__dense_activation_squared_relu__prompt_kernel(
    A_x: jax.Array,
    A_wqkv: jax.Array,
    A_wo: jax.Array,
    B_x: jax.Array,
    B_w1: jax.Array,
    B_b1: jax.Array,
    B_w2: jax.Array,
    B_b2: jax.Array,
):
    B, S, D = A_x.shape
    F = B_w1.shape[1]
    T = 512
    NQ = S // T
    assert B == 1 and D == H * DH and NQ == 4 and F % 256 == 0
    xt = jnp.swapaxes(A_x, 1, 2).reshape(D, S)
    hbm = pl.BlockSpec(memory_space=pltpu.MemorySpace.HBM)
    out = pl.pallas_call(
        functools.partial(_kernel, S=S, D=D, F=F, T=T),
        in_specs=[hbm] * 7,
        out_specs=hbm,
        out_shape=jax.ShapeDtypeStruct((D, S), A_x.dtype),
        scratch_shapes=[
            pltpu.VMEM((NQ, D, T), BF),
            pltpu.VMEM((D, 3 * D), BF),
            pltpu.VMEM((D, D), BF),
            pltpu.VMEM((D, F), BF),
            pltpu.VMEM((D, F), BF),
            pltpu.VMEM((NQ * 4, D // 2, T // 2), BF),
            pltpu.SemaphoreType.DMA((NQ + 9,)),
            pltpu.SemaphoreType.DMA(()),
            pltpu.VMEM((3 * D // 2, D), U32),
            pltpu.VMEM((7, D // 2, DP // 2), U32),
            pltpu.VMEM((7, D // 4, DP // 2), U32),
            pltpu.VMEM((D // 2, H * HP), U32),
            pltpu.VMEM((7, F // 4, DP // 2), U32),
            pltpu.VMEM((8, D // 4, F // 2), U32),
            pltpu.VMEM((D, 128), F32),
            pltpu.VMEM((D // 2 + 8, D), U32),
            pltpu.VMEM((NG * S // 2, 128), U32),
            pltpu.VMEM((NQ * D // 2, T), U32),
            pltpu.VMEM((H * HP // 2, S), U32),
            pltpu.VMEM((NQ * H * HP // 2, T), U32),
            pltpu.VMEM((S // 128, D, 128), F32),
            pltpu.VMEM((S // 128, 16, 128), F32),
            pltpu.VMEM((GH, DH * T // 16, 128), F32),
            pltpu.VMEM((NG, 160, 128), F32),
            pltpu.VMEM((GH, S, T), F32),
            pltpu.VMEM((GH, S // 2, T), U32),
            pltpu.VMEM((GH, 16, T), F32),
            pltpu.VMEM((GH, HP, T), F32),
            pltpu.VMEM((F,), BF),
            pltpu.VMEM((D,), BF),
        ],
        compiler_params=pltpu.CompilerParams(vmem_limit_bytes=100 * 1024 * 1024,
                                             disable_bounds_checks=True,
                                             disable_semaphore_checks=True),
    )(xt, A_wqkv, A_wo, B_w1, B_b1, B_w2.T, B_b2)
    return jnp.swapaxes(out.reshape(B, D, S), 1, 2)
```

```python
import functools
import math

import jax
import jax.numpy as jnp
from jax import lax
import jax.experimental.pallas as pl
import jax.experimental.pallas.tpu as pltpu

BF = jnp.bfloat16
F32 = jnp.float32
U32 = jnp.uint32

H = 16
DH = 28
HP = 32
GH = 4
NG = H // GH
GW = GH * DH
EPS = 1e-5
DP = 512
VPU_KEYS = (112, 144, 144, 128)
VPU_LATE = (4, 4, 4, 3)
VPU_MAX = 160


def _pk(x):
    return pltpu.bitcast(x, U32)


def _upk(x):
    return pltpu.bitcast(x, BF)


def _dot(a, b):
    return jnp.dot(a, b, preferred_element_type=F32)


def _after(x, dep):
    zero = (pltpu.bitcast(dep, U32) >> 31) >> 1
    zero = jnp.concatenate([zero] * (x.shape[1] // dep.shape[1]), axis=1)
    return pltpu.bitcast(pltpu.bitcast(x, U32) | zero, x.dtype)


def _rows(start, size, align):
    if isinstance(start, int):
        return pl.ds(start, size)
    return pl.ds(pl.multiple_of(start, align), size)


def _colsum(x, chains=1):
    if chains > 1:
        x = jnp.sum(x.reshape(x.shape[0] // (8 * chains), 8 * chains, x.shape[1]), axis=0)
    return jnp.sum(x, axis=0, keepdims=True)


def _shifted_moments(x, chains=1):
    inv_n = 1.0 / x.shape[0]
    d = x - x[0:1]
    dm = _colsum(d, chains) * inv_n
    var = jnp.maximum(_colsum(d * d, chains) * inv_n - dm * dm, 0.0)
    return d, dm, var


def _layernorm_t(x):
    inv_n = 1.0 / x.shape[0]
    xc = x - _colsum(x) * inv_n
    return xc * lax.rsqrt(_colsum(xc * xc) * inv_n + EPS)


def _strassen_lhs(a11, a12, a21, a22):
    return (a11 + a22, a21 + a22, a11, a22, a11 + a12, a21 - a11, a12 - a22)


def _strassen_rhs(b11, b12, b21, b22):
    return (b11 + b22, b11, b12 - b22, b21 - b11, b22, b11 + b12, b21 + b22)


def _strassen(lhs_ref, rhs, tmp, sink):
    u0, u1, u2 = tmp
    m = lambda k: _dot(_upk(lhs_ref.at[k - 1][...]), rhs[k - 1])
    u1[...] = m(5)
    z = m(3)
    sink(0, 1, u1[...] + z)
    u0[...] = z
    z = m(2)
    u0[...] = u0[...] - z
    u2[...] = z
    z = m(4)
    sink(1, 0, u2[...] + z)
    u1[...] = z - u1[...]
    u2[...] = m(1)
    z = m(7)
    sink(0, 0, u2[...] + u1[...] + z)
    z = m(6)
    sink(1, 1, u2[...] + u0[...] + z)


def _kernel(xt_hbm, wqkv_hbm, wo_hbm, w1_hbm, b1_hbm, w2t_hbm, b2_hbm, out_hbm,
            xt_v, wqkv_v, wo_v, w1_v, w2t_v, out_v, sems, osem,
            wt_s, aqk_s, av_s, wot_s, a1_s, a2_s, b2_s, wtmp_s, k_s, qt_s, vp_s, ot_s, h_s, st_s,
            qb_s, kf_s, s_s, p_s, m_s, o_s, b1_v, b2_v, *, S, D, F, T):
    NQ = S // T
    NT = T // 128
    NGI = NQ * NG
    TH, KH = T // 2, DP // 2
    qscale = (DH ** -0.5) * math.log2(math.e)

    def x_copy(b):
        return pltpu.make_async_copy(xt_hbm.at[:, pl.ds(b * T, T)], xt_v.at[b], sems.at[b])

    def w_copy(lo, hi, i):
        return pltpu.make_async_copy(wqkv_hbm.at[:, pl.ds(lo, hi - lo)],
                                     wqkv_v.at[:, pl.ds(lo, hi - lo)], sems.at[NQ + i])

    wa_copy, wb_copy = w_copy(384, 640, 0), w_copy(640, 2 * D, 1)
    wc_copy, wv_copy = w_copy(0, 384, 2), w_copy(2 * D, 3 * D, 3)
    wo_copy = pltpu.make_async_copy(wo_hbm, wo_v, sems.at[NQ + 4])
    w1_copy = pltpu.make_async_copy(w1_hbm, w1_v, sems.at[NQ + 5])
    w2_copy = pltpu.make_async_copy(w2t_hbm, w2t_v, sems.at[NQ + 6])
    b1_copy = pltpu.make_async_copy(b1_hbm, b1_v, sems.at[NQ + 7])
    b2_copy = pltpu.make_async_copy(b2_hbm, b2_v, sems.at[NQ + 8])

    for c in (wa_copy, x_copy(0), wb_copy, wc_copy, wv_copy, x_copy(1), x_copy(2), x_copy(3),
              wo_copy, w1_copy, b1_copy, b2_copy, w2_copy):
        c.start()

    def x_tile(b, n):
        return xt_v.at[b][:, pl.ds(128 * n, 128)].astype(F32)

    def store_q(b, row, col, q):
        qt_s[pl.ds((b * D + row) // 2, q.shape[0] // 2), pl.ds(col, q.shape[1])] = _pk(
            (q * qscale).astype(BF))

    def store_k(tok, kt):
        pad = jnp.zeros((128 - GW, kt.shape[1]), F32)
        for g in range(NG):
            k = jnp.concatenate([kt[GW * g:GW * (g + 1)], pad], axis=0).T.astype(BF)
            k_s[pl.ds((g * S + tok) // 2, kt.shape[1] // 2), :] = _pk(k)
            if tok == 0:
                kf_s.at[g][...] = k[:VPU_MAX].astype(F32)

    def wt_chunk(lo, n=128):
        wt = wqkv_v[:, pl.ds(lo, n)].astype(F32).T.astype(BF)
        wt_s[pl.ds(lo // 2, n // 2), :] = _pk(wt)
        return wt

    wa_copy.wait()
    wt3 = wt_chunk(384)
    wt4 = wt_chunk(512)
    x_copy(0).wait()
    xn0 = []
    for n in range(NT):
        d, dm, var = _shifted_moments(x_tile(0, n), 2)
        xn0.append(((d - dm) * lax.rsqrt(var + EPS)).astype(BF))
    xn0 = jnp.concatenate(xn0, axis=1)
    ra = _dot(jnp.concatenate([wt3, wt4], axis=0), xn0[:, :TH])
    rb = _dot(wt3, xn0[:, TH:])
    wb_copy.wait()
    wc_copy.wait()
    rc = _dot(wt4, xn0[:, TH:])
    r34 = jnp.concatenate([ra, jnp.concatenate([rb, rc], axis=0)], axis=1)
    store_q(0, 384, 0, r34[:D - 384])
    store_k(0, jnp.concatenate(
        [r34[D - 384:]] + [_dot(wt_chunk(lo), xn0) for lo in (640, 768)], axis=0))
    for lo in (0, 128):
        store_q(0, lo, 0, _dot(wt_chunk(lo), xn0))
    wt2 = wt_chunk(256)

    wv_copy.wait()
    x_copy(1).wait()
    store_q(0, 256, 0, _dot(wt2, xn0))

    def prep_lhs(dst, top, n):
        zl = jnp.zeros((n, DP - D), F32)
        t = _upk(wt_s[pl.ds(top // 2, n // 2), :]).astype(F32)
        b = _upk(wt_s[pl.ds((top + n) // 2, n // 2), :]).astype(F32)
        ops = _strassen_lhs(t[:, :KH], jnp.concatenate([t[:, KH:], zl], axis=1),
                            b[:, :KH], jnp.concatenate([b[:, KH:], zl], axis=1))
        for k in range(7):
            dst.at[k][...] = _pk(ops[k].astype(BF))

    prep_lhs(aqk_s, 0, D)
    wt_chunk(2 * D, D)
    prep_lhs(av_s, 2 * D, D // 2)

    def rhs_ops(xn):
        zr = jnp.zeros((DP - D, TH), F32)
        ops = _strassen_rhs(xn[:KH, :TH], xn[:KH, TH:],
                            jnp.concatenate([xn[KH:, :TH], zr], axis=0),
                            jnp.concatenate([xn[KH:, TH:], zr], axis=0))
        return [op.astype(BF) for op in ops]

    def ln1_ops(b):
        return rhs_ops(jnp.concatenate([_layernorm_t(x_tile(b, n)) for n in range(NT)], axis=1))

    def tmp(slot, n):
        return [s_s.at[slot, pl.ds(k * D, n), pl.ds(0, TH)] for k in range(3)]

    def qk_block(b, rhs):
        def sink(r, c, z):
            if r == 0:
                store_q(b, 0, c * TH, z)
            else:
                store_k(b * T + c * TH, z)
        _strassen(aqk_s, rhs, tmp(b % 2, D), sink)

    vtail = jnp.where(lax.broadcasted_iota(jnp.int32, (HP - DH, TH), 0) == 0, 1.0, 0.0)

    def v_block(b, rhs):
        def sink(r, c, z):
            for i in range(H // 2):
                v = jnp.concatenate([z[DH * i:DH * (i + 1)], vtail], axis=0)
                vp_s[pl.ds(HP // 2 * (r * H // 2 + i), HP // 2),
                     pl.ds(b * T + c * TH, TH)] = _pk(v.astype(BF))
        _strassen(av_s, rhs, tmp(2 + b % 2, D // 2), sink)

    rhs1 = ln1_ops(1)
    qk_block(1, rhs1)
    v_block(0, rhs_ops(xn0.astype(F32)))
    for c in (x_copy(2), x_copy(3), wo_copy, w1_copy, b1_copy):
        c.wait()
    v_block(1, rhs1)
    for b in range(2, NQ):
        rhs = ln1_ops(b)
        qk_block(b, rhs)
        v_block(b, rhs)

    prow = lax.broadcasted_iota(jnp.int32, (GW // 2, T), 0)
    qzero = jnp.zeros((64 - GW // 2, T), U32)

    def scores_mxu(gi, j, first):
        lo = DH // 2 * j
        q = qt_s[_rows(GW // 2 * gi, GW // 2, 8), :]
        q = jnp.where((prow >= lo) & (prow < lo + DH // 2), q, jnp.uint32(0))
        q = jnp.concatenate([q, qzero], axis=0)
        k = k_s[_rows((gi & (NG - 1)) * (S // 2) + first // 2, (S - first) // 2, 8), :]
        s = _dot(_upk(k), _upk(q))
        s_s.at[j][pl.ds(first, S - first), :] = s
        return s

    def scores_vpu(gi, j, r, dep=None):
        kr = kf_s.at[gi & (NG - 1)][pl.ds(r, 8), :]
        kb = jnp.concatenate([jnp.broadcast_to(kr[:, c:c + 1], (8, T))
                              for c in range(DH * j, DH * (j + 1))], axis=0)
        acc = jnp.sum((kb * qb_s.at[j][...]).reshape(DH, 8, T), axis=0)
        if dep is not None:
            acc = _after(acc, dep)
        s_s.at[j][pl.ds(r, 8), :] = acc
        return acc

    def scores(gi, j):
        s = scores_mxu(gi, j, VPU_KEYS[j])
        nr = s.shape[0] // 8
        early = VPU_KEYS[j] // 8 - VPU_LATE[j]
        skip = 40 if j == 0 else 0
        cuts = [math.ceil((u + 1) * (nr * 0.92 - skip) / early + skip) for u in range(early)]
        mx = s[:8]
        for u, (a, b) in enumerate(zip([1] + cuts, cuts + [nr])):
            seg = jnp.concatenate([mx, s[8 * a:8 * b]], axis=0)
            mx = jnp.max(seg.reshape(b - a + 1, 8, T), axis=0)
            if u < early:
                mx = jnp.maximum(mx, scores_vpu(gi, j, 8 * u))
        m_s.at[j][pl.ds(0, 8), :] = mx

    def scores_late(gi, j, o):
        m_s.at[j][pl.ds(8, 8), :] = functools.reduce(jnp.maximum, [
            scores_vpu(gi, j, VPU_KEYS[j] - 8 * (VPU_LATE[j] - u), o[:8, 128 * u:128 * (u + 1)])
            for u in range(VPU_LATE[j])])

    def spread_q(gi, j, pace=None):
        lo = DH * j // 16 * 16
        q = _upk(qt_s[_rows(GW // 2 * gi + lo // 2, 24 if j < GH - 1 else 16, 8), :]).astype(F32)
        for d in range(DH):
            r = DH * j + d - lo
            z = jnp.broadcast_to(q[r:r + 1], (8, T))
            if pace is not None:
                z = _after(z, pace[64 * d:64 * d + 8, :128])
            qb_s.at[j][pl.ds(8 * d, 8), :] = z

    def probs(j, cr=S, lo=0, hi=1):
        m = jnp.max(m_s.at[j][...], axis=0, keepdims=True)
        for c in range(lo, hi):
            p_s.at[j][pl.ds(c * cr // 2, cr // 2), :] = _pk(
                jnp.exp2(s_s.at[j][pl.ds(c * cr, cr), :] - m).astype(BF))

    def pv(gi, j):
        off = (gi & (NG - 1)) * (GH * HP // 2) + j * (HP // 2)
        o = _dot(_upk(vp_s[_rows(off, HP // 2, HP // 2), :]), _upk(p_s.at[j][...]))
        o_s.at[j][...] = o
        return o

    def normalize(gi, j):
        off = gi * (GH * HP // 2) + j * (HP // 2)
        o = o_s.at[j][...]
        o = o * (1.0 / o[DH:DH + 1, :])
        ot_s[_rows(off, HP // 2, HP // 2), :] = _pk(o.astype(BF))

    def prep_wo_w1():
        wtmp_s[pl.ds(0, D // 2), :] = _pk(wo_v[...])
        wtmp_s[pl.ds(D // 2, 8), :] = jnp.zeros((8, D), U32)
        r = lax.broadcasted_iota(jnp.int32, (HP // 2, D), 0)
        wop = jnp.concatenate(
            [jnp.where(r < DH // 2, wtmp_s[pl.ds(DH // 2 * h, HP // 2), :], jnp.uint32(0))
             for h in range(H)], axis=0)
        wot_s[...] = _pk(_upk(wop).astype(F32).T.astype(BF))
        rr = lax.broadcasted_iota(jnp.int32, (DP - D, 128), 0)
        b1 = b1_v[...].astype(F32).reshape(1, F)

        def w1t(r):
            tail = jnp.where(rr == 0, b1[:, 128 * r:128 * (r + 1)], 0.0)
            return jnp.concatenate([w1_v[:, pl.ds(128 * r, 128)].astype(F32), tail], axis=0).T

        for r in range(F // 256):
            t1, t2 = w1t(r), w1t(r + F // 256)
            ops = _strassen_lhs(t1[:, :KH], t1[:, KH:], t2[:, :KH], t2[:, KH:])
            for k in range(7):
                a1_s.at[k][pl.ds(64 * r, 64), :] = _pk(ops[k].astype(BF))

    def prep_w2(c):
        top = w2t_v[_rows(16 * c, 16, 16), :].astype(F32)
        bot = w2t_v[_rows(D // 2 + 16 * c, 16, 16), :].astype(F32)
        ops = _strassen_lhs(top[:, :F // 2], top[:, F // 2:], bot[:, :F // 2], bot[:, F // 2:])
        for k in range(7):
            a2_s.at[k][_rows(8 * c, 8, 8), :] = _pk(ops[k].astype(BF))

    def out_proj(t):
        i, n = t // NT, t % NT
        ot = _upk(ot_s[pl.ds(i * H * HP // 2, H * HP // 2), pl.ds(128 * n, 128)])
        hh = x_tile(i, n) + _dot(_upk(wot_s[...]), ot)
        h_s.at[t][...] = hh
        _, dm, var = _shifted_moments(hh)
        st_s.at[t][pl.ds(0, 8), :] = jnp.broadcast_to(hh[0:1] + dm, (8, 128))
        st_s.at[t][pl.ds(8, 8), :] = jnp.broadcast_to(var, (8, 128))

    def rstd(t):
        st_s.at[t][pl.ds(8, 8), :] = lax.rsqrt(st_s.at[t][pl.ds(8, 8), :] + EPS)

    o_s[...] = jnp.ones(o_s.shape, F32)
    for j in range(GH):
        s = scores_mxu(0, j, 0)
        m_s.at[j][...] = jnp.max(s.reshape(S // 16, 16, T), axis=0)
        spread_q(1, j, s)
        if j == 0:
            prep_wo_w1()
    w2_copy.wait()

    def body(gi, carry):
        for j in range(GH):
            normalize(jnp.maximum(gi - 1, 0), j)
            probs(j)
            scores(gi + 1, j)
            scores_late(gi + 1, j, pv(gi, j))
            spread_q(jnp.minimum(gi + 2, NGI - 1), j)
        prep_w2(jnp.minimum(gi, D // 32 - 1))
        return carry

    lax.fori_loop(0, NGI - 1, body, 0)

    gl = NGI - 1
    nfirst = (NQ - 1) * NT - 2
    nch = S // 16
    for j in range(GH):
        normalize(gl - 1, j)
    for t in range(nfirst):
        lo, hi = t * GH * nch // nfirst, (t + 1) * GH * nch // nfirst
        while lo < hi:
            j = lo // nch
            e = min(hi, (j + 1) * nch)
            probs(j, 16, lo - j * nch, e - j * nch)
            lo = e
        out_proj(t)
    b2_copy.wait()
    b2_s[...] = jnp.broadcast_to(b2_v[...].astype(F32).reshape(1, D), (128, D)).T
    for j in range(GH):
        pv(gl, j)
        normalize(gl, j)
    for t in range(nfirst):
        rstd(t)
    for t in range(nfirst, NQ * NT):
        out_proj(t)
        rstd(t)

    def out_copy(i, r, c):
        return pltpu.make_async_copy(
            out_v.at[i * 4 + r * 2 + c],
            out_hbm.at[pl.ds(r * D // 2, D // 2), _rows(i * T + c * TH, TH, TH)], osem)

    tmps = [s_s.at[k // 2, pl.ds(0, F // 2), pl.ds(k % 2 * TH, TH)] for k in range(6)]
    ab = [p_s.at[k // 2, pl.ds(0, F // 4), pl.ds(k % 2 * TH, TH)] for k in range(7)]
    htail = jnp.where(lax.broadcasted_iota(jnp.int32, (DP - D, TH), 0) == 0, 1.0, 0.0)

    def ffn(i, carry):
        def hn(r, c):
            lo, hi = r * KH, min((r + 1) * KH, D)
            cols = []
            for n in range(NT // 2):
                t = i * NT + c * NT // 2 + n
                z = h_s.at[t][pl.ds(lo, hi - lo), :].reshape((hi - lo) // 8, 8, 128)
                z = (z - st_s.at[t][pl.ds(0, 8), :]) * st_s.at[t][pl.ds(8, 8), :]
                cols.append(z.reshape(hi - lo, 128))
            z = jnp.concatenate(cols, axis=1)
            return z if r == 0 else jnp.concatenate([z, htail], axis=0)

        a11, a12, a21 = tmps[3:]

        def put(k, val):
            ab[k - 1][...] = _pk(val.astype(BF))

        def sink(r, c, z):
            a = jnp.square(jnp.maximum(z, 0.0))
            if (r, c) == (0, 1):
                a12[...] = a
            elif (r, c) == (1, 0):
                a21[...] = a
            elif (r, c) == (0, 0):
                a11[...] = a
                put(2, a)
                put(4, a21[...] - a)
                put(6, a + a12[...])
            else:
                put(1, a11[...] + a)
                put(3, a12[...] - a)
                put(5, a)
                put(7, a21[...] + a)

        rhs = [op.astype(BF) for op in _strassen_rhs(hn(0, 0), hn(0, 1), hn(1, 0), hn(1, 1))]
        _strassen(a1_s, rhs, tmps[:3], sink)

        def emit(r, c, y):
            rows = pl.ds(r * D // 2, D // 2)
            hh = jnp.concatenate(
                [h_s.at[i * NT + c * NT // 2 + n][rows, :] + b2_s[rows, :] for n in range(NT // 2)],
                axis=1)
            out_v.at[i * 4 + r * 2 + c][...] = (hh + y).astype(BF)
            out_copy(i, r, c).start()

        m = lambda k: _dot(_upk(a2_s.at[k - 1][...]), _upk(ab[k - 1][...]))
        m2, m4 = m(2), m(4)
        emit(1, 0, m2 + m4)
        m6, m1, m3 = m(6), m(1), m(3)
        emit(1, 1, m1 - m2 + m3 + m6)
        m5 = m(5)
        emit(0, 1, m3 + m5)
        m7 = m(7)
        emit(0, 0, m1 + m4 - m5 + m7)
        return carry

    lax.fori_loop(0, NQ, ffn, 0)
    for i in range(NQ):
        for r in range(2):
            for c in range(2):
                out_copy(i, r, c).wait()


@jax.jit
def pallas_sequential_preLN__mha_block__dense_activation_squared_relu__prompt_kernel(
    A_x: jax.Array,
    A_wqkv: jax.Array,
    A_wo: jax.Array,
    B_x: jax.Array,
    B_w1: jax.Array,
    B_b1: jax.Array,
    B_w2: jax.Array,
    B_b2: jax.Array,
):
    B, S, D = A_x.shape
    F = B_w1.shape[1]
    T = 512
    NQ = S // T
    assert B == 1 and D == H * DH and NQ == 4 and F % 256 == 0
    xt = jnp.swapaxes(A_x, 1, 2).reshape(D, S)
    hbm = pl.BlockSpec(memory_space=pltpu.MemorySpace.HBM)
    out = pl.pallas_call(
        functools.partial(_kernel, S=S, D=D, F=F, T=T),
        in_specs=[hbm] * 7,
        out_specs=hbm,
        out_shape=jax.ShapeDtypeStruct((D, S), A_x.dtype),
        scratch_shapes=[
            pltpu.VMEM((NQ, D, T), BF),
            pltpu.VMEM((D, 3 * D), BF),
            pltpu.VMEM((D, D), BF),
            pltpu.VMEM((D, F), BF),
            pltpu.VMEM((D, F), BF),
            pltpu.VMEM((NQ * 4, D // 2, T // 2), BF),
            pltpu.SemaphoreType.DMA((NQ + 9,)),
            pltpu.SemaphoreType.DMA(()),
            pltpu.VMEM((3 * D // 2, D), U32),
            pltpu.VMEM((7, D // 2, DP // 2), U32),
            pltpu.VMEM((7, D // 4, DP // 2), U32),
            pltpu.VMEM((D // 2, H * HP), U32),
            pltpu.VMEM((7, F // 4, DP // 2), U32),
            pltpu.VMEM((8, D // 4, F // 2), U32),
            pltpu.VMEM((D, 128), F32),
            pltpu.VMEM((D // 2 + 8, D), U32),
            pltpu.VMEM((NG * S // 2, 128), U32),
            pltpu.VMEM((NQ * D // 2, T), U32),
            pltpu.VMEM((H * HP // 2, S), U32),
            pltpu.VMEM((NQ * H * HP // 2, T), U32),
            pltpu.VMEM((S // 128, D, 128), F32),
            pltpu.VMEM((S // 128, 16, 128), F32),
            pltpu.VMEM((GH, DH * 8, T), F32),
            pltpu.VMEM((NG, VPU_MAX, 128), F32),
            pltpu.VMEM((GH, S, T), F32),
            pltpu.VMEM((GH, S // 2, T), U32),
            pltpu.VMEM((GH, 16, T), F32),
            pltpu.VMEM((GH, HP, T), F32),
            pltpu.VMEM((F,), BF),
            pltpu.VMEM((D,), BF),
        ],
        compiler_params=pltpu.CompilerParams(vmem_limit_bytes=100 * 1024 * 1024,
                                             disable_bounds_checks=True,
                                             disable_semaphore_checks=True),
    )(xt, A_wqkv, A_wo, B_w1, B_b1, B_w2.T, B_b2)
    return jnp.swapaxes(out.reshape(B, D, S), 1, 2)
```

```python
import functools
import math

import jax
import jax.numpy as jnp
from jax import lax
import jax.experimental.pallas as pl
import jax.experimental.pallas.tpu as pltpu

BF = jnp.bfloat16
F32 = jnp.float32
U32 = jnp.uint32

H = 16
DH = 28
HP = 32
GH = 4
NG = H // GH
GW = GH * DH
EPS = 1e-5
DP = 512
VPU_KEYS = (112, 144, 144, 128)
VPU_LATE = (4, 4, 4, 3)
VPU_MAX = 160


def _pk(x):
    return pltpu.bitcast(x, U32)


def _upk(x):
    return pltpu.bitcast(x, BF)


def _dot(a, b):
    return jnp.dot(a, b, preferred_element_type=F32)


def _after(x, dep):
    zero = (pltpu.bitcast(dep, U32) >> 31) >> 1
    zero = jnp.concatenate([zero] * (x.shape[1] // dep.shape[1]), axis=1)
    return pltpu.bitcast(pltpu.bitcast(x, U32) | zero, x.dtype)


def _rows(start, size, align):
    if isinstance(start, int):
        return pl.ds(start, size)
    return pl.ds(pl.multiple_of(start, align), size)


def _colsum(x, chains=1):
    if chains > 1:
        x = jnp.sum(x.reshape(x.shape[0] // (8 * chains), 8 * chains, x.shape[1]), axis=0)
    return jnp.sum(x, axis=0, keepdims=True)


def _shifted_moments(x, chains=1):
    inv_n = 1.0 / x.shape[0]
    d = x - x[0:1]
    dm = _colsum(d, chains) * inv_n
    var = jnp.maximum(_colsum(d * d, chains) * inv_n - dm * dm, 0.0)
    return d, dm, var


def _layernorm_t(x):
    inv_n = 1.0 / x.shape[0]
    xc = x - _colsum(x) * inv_n
    rstd = lax.rsqrt(_colsum(xc * xc) * inv_n + EPS)
    return xc * rstd, rstd


def _strassen_lhs(a11, a12, a21, a22):
    return (a11 + a22, a21 + a22, a11, a22, a11 + a12, a21 - a11, a12 - a22)


def _strassen_rhs(b11, b12, b21, b22):
    return (b11 + b22, b11, b12 - b22, b21 - b11, b22, b11 + b12, b21 + b22)


def _strassen(lhs_ref, rhs, tmp, sink, deps=None):
    u0, u1, u2 = tmp

    def m(k):
        z = _dot(_upk(lhs_ref.at[k - 1][...]), rhs[k - 1])
        if deps and k in deps:
            r = z.shape[0] // 16 * 8
            z = jnp.concatenate([z[:r], _after(z[r:r + 8], deps[k]), z[r + 8:]], axis=0)
        return z

    u1[...] = m(5)
    z = m(3)
    sink(0, 1, u1[...] + z)
    u0[...] = z
    z = m(2)
    u0[...] = u0[...] - z
    u2[...] = z
    z = m(4)
    sink(1, 0, u2[...] + z)
    u1[...] = z - u1[...]
    u2[...] = m(1)
    z = m(7)
    sink(0, 0, u2[...] + u1[...] + z)
    z = m(6)
    sink(1, 1, u2[...] + u0[...] + z)


def _kernel(xt_hbm, wqkv_hbm, wo_hbm, w1_hbm, b1_hbm, w2t_hbm, b2_hbm, out_hbm,
            xt_v, wqkv_v, wo_v, w1_v, w2t_v, out_v, sems, osem,
            wt_s, aqk_s, av_s, wot_s, a1_s, a2_s, b2_s, wtmp_s, k_s, qt_s, vp_s, ot_s,
            h_s, st_s, raw_s, qb_s, kf_s, s_s, p_s, m_s, o_s, b1_v, b2_v, *, S, D, F, T):
    NQ = S // T
    NT = T // 128
    NGI = NQ * NG
    TH, KH = T // 2, DP // 2
    qscale = (DH ** -0.5) * math.log2(math.e)

    def x_copy(b):
        return pltpu.make_async_copy(xt_hbm.at[:, pl.ds(b * T, T)], xt_v.at[b], sems.at[b])

    def x0_copy(n):
        cols = pl.ds(0, 128) if n == 0 else pl.ds(128, T - 128)
        return pltpu.make_async_copy(xt_hbm.at[:, cols], xt_v.at[0, :, cols],
                                     sems.at[NQ + 9 if n else 0])

    def w_copy(lo, hi, i):
        return pltpu.make_async_copy(wqkv_hbm.at[:, pl.ds(lo, hi - lo)],
                                     wqkv_v.at[:, pl.ds(lo, hi - lo)], sems.at[NQ + i])

    wa_copy, wb_copy = w_copy(384, 640, 0), w_copy(640, 2 * D, 1)
    wc_copy, wv_copy = w_copy(0, 384, 2), w_copy(2 * D, 3 * D, 3)
    wo_copy = pltpu.make_async_copy(wo_hbm, wo_v, sems.at[NQ + 4])
    w1_copy = pltpu.make_async_copy(w1_hbm, w1_v, sems.at[NQ + 5])
    w2_copy = pltpu.make_async_copy(w2t_hbm, w2t_v, sems.at[NQ + 6])
    b1_copy = pltpu.make_async_copy(b1_hbm, b1_v, sems.at[NQ + 7])
    b2_copy = pltpu.make_async_copy(b2_hbm, b2_v, sems.at[NQ + 8])

    for c in (wa_copy, x0_copy(0), x0_copy(1), wb_copy, wc_copy, wv_copy,
              x_copy(1), x_copy(2), x_copy(3), wo_copy, w1_copy, b1_copy, b2_copy, w2_copy):
        c.start()

    def x_tile(b, n):
        return xt_v.at[b][:, pl.ds(128 * n, 128)].astype(F32)

    def store_q(b, row, col, q):
        qt_s[pl.ds((b * D + row) // 2, q.shape[0] // 2), pl.ds(col, q.shape[1])] = _pk(
            (q * qscale).astype(BF))

    def store_k(tok, kt):
        pad = jnp.zeros((128 - GW, kt.shape[1]), F32)
        for g in range(NG):
            k = jnp.concatenate([kt[GW * g:GW * (g + 1)], pad], axis=0).T.astype(BF)
            k_s[pl.ds((g * S + tok) // 2, kt.shape[1] // 2), :] = _pk(k)
            if tok == 0:
                kf_s.at[g][...] = k[:VPU_MAX].astype(F32)

    def wt_chunk(lo, n=128):
        wt = wqkv_v[:, pl.ds(lo, n)].astype(F32).T.astype(BF)
        wt_s[pl.ds(lo // 2, n // 2), :] = _pk(wt)
        return wt

    wa_copy.wait()
    x0_copy(0).wait()
    wt3 = wt_chunk(384)
    wt4 = wt_chunk(512)
    xn0 = []
    for n in range(NT):
        if n == 1:
            x0_copy(1).wait()
        d, dm, var = _shifted_moments(x_tile(0, n), 2)
        xn0.append(((d - dm) * lax.rsqrt(var + EPS)).astype(BF))
    xn0 = jnp.concatenate(xn0, axis=1)
    ra = _dot(jnp.concatenate([wt3, wt4], axis=0), xn0[:, :T - 128])
    rb = _dot(wt3, xn0[:, T - 128:])
    wb_copy.wait()
    wc_copy.wait()
    rc = _dot(wt4, xn0[:, T - 128:])
    r34 = jnp.concatenate([ra, jnp.concatenate([rb, rc], axis=0)], axis=1)
    store_q(0, 384, 0, r34[:D - 384])
    store_k(0, jnp.concatenate(
        [r34[D - 384:]] + [_dot(wt_chunk(lo), xn0) for lo in (640, 768)], axis=0))
    for lo in (0, 128):
        store_q(0, lo, 0, _dot(wt_chunk(lo), xn0))
    wt2 = wt_chunk(256)

    wv_copy.wait()
    x_copy(1).wait()
    store_q(0, 256, 0, _dot(wt2, xn0))

    def prep_lhs(dst, top, n):
        zl = jnp.zeros((n, DP - D), F32)
        t = _upk(wt_s[pl.ds(top // 2, n // 2), :]).astype(F32)
        b = _upk(wt_s[pl.ds((top + n) // 2, n // 2), :]).astype(F32)
        ops = _strassen_lhs(t[:, :KH], jnp.concatenate([t[:, KH:], zl], axis=1),
                            b[:, :KH], jnp.concatenate([b[:, KH:], zl], axis=1))
        for k in range(7):
            dst.at[k][...] = _pk(ops[k].astype(BF))

    prep_lhs(aqk_s, 0, D)
    wt_chunk(2 * D, D)
    prep_lhs(av_s, 2 * D, D // 2)

    def rhs_ops(xn):
        zr = jnp.zeros((DP - D, TH), F32)
        ops = _strassen_rhs(xn[:KH, :TH], xn[:KH, TH:],
                            jnp.concatenate([xn[KH:, :TH], zr], axis=0),
                            jnp.concatenate([xn[KH:, TH:], zr], axis=0))
        return [op.astype(BF) for op in ops]

    def ln1_ops(b):
        res = [_layernorm_t(x_tile(b, n)) for n in range(NT)]
        return (rhs_ops(jnp.concatenate([z for z, _ in res], axis=1)),
                [jnp.broadcast_to(r, (8, 128)) for _, r in res])

    def tmp(slot, n):
        return [s_s.at[slot, pl.ds(k * D, n), pl.ds(0, TH)] for k in range(3)]

    def qk_block(b, rhs, deps=None):
        def sink(r, c, z):
            if r == 0:
                store_q(b, 0, c * TH, z)
            else:
                store_k(b * T + c * TH, z)
        _strassen(aqk_s, rhs, tmp(b % 2, D), sink, deps)

    vtail = jnp.where(lax.broadcasted_iota(jnp.int32, (HP - DH, TH), 0) == 0, 1.0, 0.0)

    def v_block(b, rhs, deps=None):
        def sink(r, c, z):
            for i in range(H // 2):
                v = jnp.concatenate([z[DH * i:DH * (i + 1)], vtail], axis=0)
                vp_s[pl.ds(HP // 2 * (r * H // 2 + i), HP // 2),
                     pl.ds(b * T + c * TH, TH)] = _pk(v.astype(BF))
        _strassen(av_s, rhs, tmp(2 + b % 2, D // 2), sink, deps)

    rhs1, r1 = ln1_ops(1)
    qk_block(1, rhs1, {5: r1[0]})
    v_block(0, rhs_ops(xn0.astype(F32)))
    for c in (x_copy(2), x_copy(3), wo_copy, w1_copy, b1_copy):
        c.wait()
    rhs_prev = rhs1
    for b in range(2, NQ):
        rhs, r = ln1_ops(b)
        v_block(b - 1, rhs_prev, {3: r[2], 4: r[3], 7: r[0]})
        qk_block(b, rhs, {5: r[1]})
        rhs_prev = rhs
    v_block(NQ - 1, rhs_prev)

    prow = lax.broadcasted_iota(jnp.int32, (GW // 2, T), 0)
    qzero = jnp.zeros((64 - GW // 2, T), U32)

    def scores_mxu(gi, j, first):
        lo = DH // 2 * j
        q = qt_s[_rows(GW // 2 * gi, GW // 2, 8), :]
        q = jnp.where((prow >= lo) & (prow < lo + DH // 2), q, jnp.uint32(0))
        q = jnp.concatenate([q, qzero], axis=0)
        k = k_s[_rows((gi & (NG - 1)) * (S // 2) + first // 2, (S - first) // 2, 8), :]
        s = _dot(_upk(k), _upk(q))
        s_s.at[j][pl.ds(first, S - first), :] = s
        return s

    def scores_vpu(gi, j, r, dep=None):
        kr = kf_s.at[gi & (NG - 1)][pl.ds(r, 8), :]
        kb = jnp.concatenate([jnp.broadcast_to(kr[:, c:c + 1], (8, T))
                              for c in range(DH * j, DH * (j + 1))], axis=0)
        acc = jnp.sum((kb * qb_s.at[j][...]).reshape(DH, 8, T), axis=0)
        if dep is not None:
            acc = _after(acc, dep)
        s_s.at[j][pl.ds(r, 8), :] = acc
        return acc

    def scores(gi, j):
        s = scores_mxu(gi, j, VPU_KEYS[j])
        nr = s.shape[0] // 8
        early = VPU_KEYS[j] // 8 - VPU_LATE[j]
        skip = 40 if j == 0 else 0
        cuts = [math.ceil((u + 1) * (nr * 0.92 - skip) / early + skip) for u in range(early)]
        mx = s[:8]
        for u, (a, b) in enumerate(zip([1] + cuts, cuts + [nr])):
            seg = jnp.concatenate([mx, s[8 * a:8 * b]], axis=0)
            mx = jnp.max(seg.reshape(b - a + 1, 8, T), axis=0)
            if u < early:
                mx = jnp.maximum(mx, scores_vpu(gi, j, 8 * u))
        m_s.at[j][pl.ds(0, 8), :] = mx

    def scores_late(gi, j, o):
        m_s.at[j][pl.ds(8, 8), :] = functools.reduce(jnp.maximum, [
            scores_vpu(gi, j, VPU_KEYS[j] - 8 * (VPU_LATE[j] - u), o[:8, 128 * u:128 * (u + 1)])
            for u in range(VPU_LATE[j])])

    def spread_q(gi, j, pace=None):
        lo = DH * j // 16 * 16
        q = _upk(qt_s[_rows(GW // 2 * gi + lo // 2, 24 if j < GH - 1 else 16, 8), :]).astype(F32)
        for d in range(DH):
            r = DH * j + d - lo
            z = jnp.broadcast_to(q[r:r + 1], (8, T))
            if pace is not None:
                z = _after(z, pace[64 * d:64 * d + 8, :128])
            qb_s.at[j][pl.ds(8 * d, 8), :] = z

    def probs(j, cr=S, lo=0, hi=1):
        m = jnp.max(m_s.at[j][...], axis=0, keepdims=True)
        for c in range(lo, hi):
            p_s.at[j][pl.ds(c * cr // 2, cr // 2), :] = _pk(
                jnp.exp2(s_s.at[j][pl.ds(c * cr, cr), :] - m).astype(BF))

    def pv(gi, j):
        off = (gi & (NG - 1)) * (GH * HP // 2) + j * (HP // 2)
        o = _dot(_upk(vp_s[_rows(off, HP // 2, HP // 2), :]), _upk(p_s.at[j][...]))
        o_s.at[j][...] = o
        return o

    def normalize(gi, j):
        off = gi * (GH * HP // 2) + j * (HP // 2)
        o = o_s.at[j][...]
        o = o * (1.0 / o[DH:DH + 1, :])
        ot_s[_rows(off, HP // 2, HP // 2), :] = _pk(o.astype(BF))

    def prep_wo_w1():
        wtmp_s[pl.ds(0, D // 2), :] = _pk(wo_v[...])
        wtmp_s[pl.ds(D // 2, 8), :] = jnp.zeros((8, D), U32)
        r = lax.broadcasted_iota(jnp.int32, (HP // 2, D), 0)
        wop = jnp.concatenate(
            [jnp.where(r < DH // 2, wtmp_s[pl.ds(DH // 2 * h, HP // 2), :], jnp.uint32(0))
             for h in range(H)], axis=0)
        wot_s[...] = _pk(_upk(wop).astype(F32).T.astype(BF))
        rr = lax.broadcasted_iota(jnp.int32, (DP - D, 128), 0)
        b1 = b1_v[...].astype(F32).reshape(1, F)

        def w1t(r):
            tail = jnp.where(rr == 0, b1[:, 128 * r:128 * (r + 1)], 0.0)
            return jnp.concatenate([w1_v[:, pl.ds(128 * r, 128)].astype(F32), tail], axis=0).T

        for r in range(F // 256):
            t1, t2 = w1t(r), w1t(r + F // 256)
            ops = _strassen_lhs(t1[:, :KH], t1[:, KH:], t2[:, :KH], t2[:, KH:])
            for k in range(7):
                a1_s.at[k][pl.ds(64 * r, 64), :] = _pk(ops[k].astype(BF))

    def prep_w2(c):
        top = w2t_v[_rows(16 * c, 16, 16), :].astype(F32)
        bot = w2t_v[_rows(D // 2 + 16 * c, 16, 16), :].astype(F32)
        ops = _strassen_lhs(top[:, :F // 2], top[:, F // 2:], bot[:, :F // 2], bot[:, F // 2:])
        for k in range(7):
            a2_s.at[k][_rows(8 * c, 8, 8), :] = _pk(ops[k].astype(BF))

    def out_proj(t):
        i, n = t // NT, t % NT
        ot = _upk(ot_s[pl.ds(i * H * HP // 2, H * HP // 2), pl.ds(128 * n, 128)])
        hh = x_tile(i, n) + _dot(_upk(wot_s[...]), ot)
        h_s.at[t][...] = hh
        d = (hh - hh[0:1]).reshape(D // 8, 8, 128)
        raw_s.at[t][pl.ds(0, 8), :] = jnp.sum(d, axis=0)
        raw_s.at[t][pl.ds(8, 8), :] = jnp.sum(d * d, axis=0)

    def ln2_stats(i, dep=None):
        for n in range(NT):
            t = i * NT + n
            s1, s2 = raw_s.at[t][pl.ds(0, 8), :], raw_s.at[t][pl.ds(8, 8), :]
            if dep is not None:
                s1, s2 = _after(s1, dep), _after(s2, dep)
            dm = jnp.sum(s1, axis=0, keepdims=True) * (1.0 / D)
            var = jnp.sum(s2, axis=0, keepdims=True) * (1.0 / D) - dm * dm
            rstd = lax.rsqrt(jnp.maximum(var, 0.0) + EPS)
            st_s.at[t][pl.ds(0, 8), :] = jnp.broadcast_to(h_s.at[t][pl.ds(0, 1), :] + dm, (8, 128))
            st_s.at[t][pl.ds(8, 8), :] = jnp.broadcast_to(rstd, (8, 128))

    o_s[...] = jnp.ones(o_s.shape, F32)
    for j in range(GH):
        s = scores_mxu(0, j, 0)
        m_s.at[j][...] = jnp.max(s.reshape(S // 16, 16, T), axis=0)
        spread_q(1, j, s)
        if j == 0:
            prep_wo_w1()
    w2_copy.wait()

    def body(gi, carry):
        for j in range(GH):
            normalize(jnp.maximum(gi - 1, 0), j)
            probs(j)
            scores(gi + 1, j)
            scores_late(gi + 1, j, pv(gi, j))
            spread_q(jnp.minimum(gi + 2, NGI - 1), j)
        prep_w2(jnp.minimum(gi, D // 32 - 1))
        return carry

    lax.fori_loop(0, NGI - 1, body, 0)

    gl = NGI - 1
    nfirst = (NQ - 1) * NT - 2
    nch = S // 16
    for j in range(GH):
        normalize(gl - 1, j)
    for t in range(nfirst):
        lo, hi = t * GH * nch // nfirst, (t + 1) * GH * nch // nfirst
        while lo < hi:
            j = lo // nch
            e = min(hi, (j + 1) * nch)
            probs(j, 16, lo - j * nch, e - j * nch)
            lo = e
        out_proj(t)
    b2_copy.wait()
    b2_s[...] = jnp.broadcast_to(b2_v[...].astype(F32).reshape(1, D), (128, D)).T
    for j in range(GH):
        pv(gl, j)
        normalize(gl, j)
    ln2_stats(0)
    for t in range(nfirst, NQ * NT):
        out_proj(t)

    def out_copy(i, r, c):
        return pltpu.make_async_copy(
            out_v.at[i * 4 + r * 2 + c],
            out_hbm.at[pl.ds(r * D // 2, D // 2), _rows(i * T + c * TH, TH, TH)], osem)

    tmps = [s_s.at[k // 2, pl.ds(0, F // 2), pl.ds(k % 2 * TH, TH)] for k in range(6)]
    ab = [p_s.at[k // 2, pl.ds(0, F // 4), pl.ds(k % 2 * TH, TH)] for k in range(7)]
    htail = jnp.where(lax.broadcasted_iota(jnp.int32, (DP - D, TH), 0) == 0, 1.0, 0.0)

    def ffn(i, carry):
        def hn(r, c):
            lo, hi = r * KH, min((r + 1) * KH, D)
            cols = []
            for n in range(NT // 2):
                t = i * NT + c * NT // 2 + n
                z = h_s.at[t][pl.ds(lo, hi - lo), :].reshape((hi - lo) // 8, 8, 128)
                z = (z - st_s.at[t][pl.ds(0, 8), :]) * st_s.at[t][pl.ds(8, 8), :]
                cols.append(z.reshape(hi - lo, 128))
            z = jnp.concatenate(cols, axis=1)
            return z if r == 0 else jnp.concatenate([z, htail], axis=0)

        a11, a12, a21 = tmps[3:]

        def put(k, val):
            ab[k - 1][...] = _pk(val.astype(BF))

        def sink(r, c, z):
            a = jnp.square(jnp.maximum(z, 0.0))
            if (r, c) == (0, 1):
                a12[...] = a
            elif (r, c) == (1, 0):
                a21[...] = a
            elif (r, c) == (0, 0):
                a11[...] = a
                put(2, a)
                put(4, a21[...] - a)
                put(6, a + a12[...])
            else:
                put(1, a11[...] + a)
                put(3, a12[...] - a)
                put(5, a)
                put(7, a21[...] + a)

        rhs = [op.astype(BF) for op in _strassen_rhs(hn(0, 0), hn(0, 1), hn(1, 0), hn(1, 1))]
        _strassen(a1_s, rhs, tmps[:3], sink)

        def emit(r, c, y):
            rows = pl.ds(r * D // 2, D // 2)
            hh = jnp.concatenate(
                [h_s.at[i * NT + c * NT // 2 + n][rows, :] + b2_s[rows, :] for n in range(NT // 2)],
                axis=1)
            out_v.at[i * 4 + r * 2 + c][...] = (hh + y).astype(BF)
            out_copy(i, r, c).start()

        m = lambda k: _dot(_upk(a2_s.at[k - 1][...]), _upk(ab[k - 1][...]))
        m2, m4 = m(2), m(4)
        ln2_stats(jnp.minimum(i + 1, NQ - 1), m2[:8, :128])
        emit(1, 0, m2 + m4)
        m6, m1, m3 = m(6), m(1), m(3)
        emit(1, 1, m1 - m2 + m3 + m6)
        m5 = m(5)
        emit(0, 1, m3 + m5)
        m7 = m(7)
        emit(0, 0, m1 + m4 - m5 + m7)
        return carry

    lax.fori_loop(0, NQ, ffn, 0)
    for i in range(NQ):
        for r in range(2):
            for c in range(2):
                out_copy(i, r, c).wait()


@jax.jit
def pallas_sequential_preLN__mha_block__dense_activation_squared_relu__prompt_kernel(
    A_x: jax.Array,
    A_wqkv: jax.Array,
    A_wo: jax.Array,
    B_x: jax.Array,
    B_w1: jax.Array,
    B_b1: jax.Array,
    B_w2: jax.Array,
    B_b2: jax.Array,
):
    B, S, D = A_x.shape
    F = B_w1.shape[1]
    T = 512
    NQ = S // T
    assert B == 1 and D == H * DH and NQ == 4 and F % 256 == 0
    xt = jnp.swapaxes(A_x, 1, 2).reshape(D, S)
    hbm = pl.BlockSpec(memory_space=pltpu.MemorySpace.HBM)
    out = pl.pallas_call(
        functools.partial(_kernel, S=S, D=D, F=F, T=T),
        in_specs=[hbm] * 7,
        out_specs=hbm,
        out_shape=jax.ShapeDtypeStruct((D, S), A_x.dtype),
        scratch_shapes=[
            pltpu.VMEM((NQ, D, T), BF),
            pltpu.VMEM((D, 3 * D), BF),
            pltpu.VMEM((D, D), BF),
            pltpu.VMEM((D, F), BF),
            pltpu.VMEM((D, F), BF),
            pltpu.VMEM((NQ * 4, D // 2, T // 2), BF),
            pltpu.SemaphoreType.DMA((NQ + 10,)),
            pltpu.SemaphoreType.DMA(()),
            pltpu.VMEM((3 * D // 2, D), U32),
            pltpu.VMEM((7, D // 2, DP // 2), U32),
            pltpu.VMEM((7, D // 4, DP // 2), U32),
            pltpu.VMEM((D // 2, H * HP), U32),
            pltpu.VMEM((7, F // 4, DP // 2), U32),
            pltpu.VMEM((8, D // 4, F // 2), U32),
            pltpu.VMEM((D, 128), F32),
            pltpu.VMEM((D // 2 + 8, D), U32),
            pltpu.VMEM((NG * S // 2, 128), U32),
            pltpu.VMEM((NQ * D // 2, T), U32),
            pltpu.VMEM((H * HP // 2, S), U32),
            pltpu.VMEM((NQ * H * HP // 2, T), U32),
            pltpu.VMEM((S // 128, D, 128), F32),
            pltpu.VMEM((S // 128, 16, 128), F32),
            pltpu.VMEM((S // 128, 16, 128), F32),
            pltpu.VMEM((GH, DH * 8, T), F32),
            pltpu.VMEM((NG, VPU_MAX, 128), F32),
            pltpu.VMEM((GH, S, T), F32),
            pltpu.VMEM((GH, S // 2, T), U32),
            pltpu.VMEM((GH, 16, T), F32),
            pltpu.VMEM((GH, HP, T), F32),
            pltpu.VMEM((F,), BF),
            pltpu.VMEM((D,), BF),
        ],
        compiler_params=pltpu.CompilerParams(vmem_limit_bytes=100 * 1024 * 1024,
                                             disable_bounds_checks=True,
                                             disable_semaphore_checks=True),
    )(xt, A_wqkv, A_wo, B_w1, B_b1, B_w2.T, B_b2)
    return jnp.swapaxes(out.reshape(B, D, S), 1, 2)
```

```python
import functools
import math

import jax
import jax.numpy as jnp
from jax import lax
import jax.experimental.pallas as pl
import jax.experimental.pallas.tpu as pltpu

BF = jnp.bfloat16
F32 = jnp.float32
U32 = jnp.uint32

H = 16
DH = 28
HP = 32
GH = 4
NG = H // GH
GW = GH * DH
EPS = 1e-5
DP = 512
VPU_KEYS = (112, 144, 144, 144)
VPU_LATE = (4, 4, 4, 4)
VPU_SPAN = ((26, 0.92), (-4, 0.961), (-5, 0.959), (-8, 0.944))
VPU_MAX = 160


def _pk(x):
    return pltpu.bitcast(x, U32)


def _upk(x):
    return pltpu.bitcast(x, BF)


def _dot(a, b):
    return jnp.dot(a, b, preferred_element_type=F32)


def _after(x, dep):
    zero = (pltpu.bitcast(dep, U32) >> 31) >> 1
    zero = jnp.concatenate([zero] * (x.shape[1] // dep.shape[1]), axis=1)
    return pltpu.bitcast(pltpu.bitcast(x, U32) | zero, x.dtype)


def _rows(start, size, align):
    if isinstance(start, int):
        return pl.ds(start, size)
    return pl.ds(pl.multiple_of(start, align), size)


def _colsum(x, chains=1):
    if chains > 1:
        x = jnp.sum(x.reshape(x.shape[0] // (8 * chains), 8 * chains, x.shape[1]), axis=0)
    return jnp.sum(x, axis=0, keepdims=True)


def _shifted_moments(x, chains=1):
    inv_n = 1.0 / x.shape[0]
    d = x - x[0:1]
    dm = _colsum(d, chains) * inv_n
    var = jnp.maximum(_colsum(d * d, chains) * inv_n - dm * dm, 0.0)
    return d, dm, var


def _layernorm_t(x):
    inv_n = 1.0 / x.shape[0]
    xc = x - _colsum(x) * inv_n
    rstd = lax.rsqrt(_colsum(xc * xc) * inv_n + EPS)
    return xc * rstd, rstd


def _strassen_lhs(a11, a12, a21, a22):
    return (a11 + a22, a21 + a22, a11, a22, a11 + a12, a21 - a11, a12 - a22)


def _strassen_rhs(b11, b12, b21, b22):
    return (b11 + b22, b11, b12 - b22, b21 - b11, b22, b11 + b12, b21 + b22)


def _strassen(lhs_ref, rhs, tmp, sink, deps=None):
    u0, u1, u2 = tmp

    def m(k):
        z = _dot(_upk(lhs_ref.at[k - 1][...]), rhs[k - 1])
        if deps and k in deps:
            r = z.shape[0] // 16 * 8
            z = jnp.concatenate([z[:r], _after(z[r:r + 8], deps[k]), z[r + 8:]], axis=0)
        return z

    u1[...] = m(5)
    z = m(3)
    sink(0, 1, u1[...] + z)
    u0[...] = z
    z = m(2)
    u0[...] = u0[...] - z
    u2[...] = z
    z = m(4)
    sink(1, 0, u2[...] + z)
    u1[...] = z - u1[...]
    u2[...] = m(1)
    z = m(7)
    sink(0, 0, u2[...] + u1[...] + z)
    z = m(6)
    sink(1, 1, u2[...] + u0[...] + z)


def _kernel(xt_hbm, wqkv_hbm, wo_hbm, w1_hbm, b1_hbm, w2t_hbm, b2_hbm, out_hbm,
            xt_v, wqkv_v, wo_v, w1_v, w2t_v, out_v, sems, osem,
            wt_s, aqk_s, av_s, wot_s, a1_s, a2_s, b2_s, wtmp_s, k_s, qt_s, vp_s, ot_s,
            h_s, st_s, raw_s, first_s, qb_s, kf_s, s_s, p_s, m_s, o_s, b1_v, b2_v, *, S, D, F, T):
    NQ = S // T
    NT = T // 128
    NGI = NQ * NG
    TH, KH = T // 2, DP // 2
    qscale = (DH ** -0.5) * math.log2(math.e)

    def x_copy(b):
        return pltpu.make_async_copy(xt_hbm.at[:, pl.ds(b * T, T)], xt_v.at[b], sems.at[b])

    def x0_copy(n):
        cols = pl.ds(0, 128) if n == 0 else pl.ds(128, T - 128)
        return pltpu.make_async_copy(xt_hbm.at[:, cols], xt_v.at[0, :, cols],
                                     sems.at[NQ + 9 if n else 0])

    def w_copy(lo, hi, i):
        return pltpu.make_async_copy(wqkv_hbm.at[:, pl.ds(lo, hi - lo)],
                                     wqkv_v.at[:, pl.ds(lo, hi - lo)], sems.at[NQ + i])

    wa_copy, wb_copy = w_copy(384, 640, 0), w_copy(640, 2 * D, 1)
    wc_copy, wv_copy = w_copy(0, 384, 2), w_copy(2 * D, 3 * D, 3)
    wo_copy = pltpu.make_async_copy(wo_hbm, wo_v, sems.at[NQ + 4])
    w1_copy = pltpu.make_async_copy(w1_hbm, w1_v, sems.at[NQ + 5])
    w2_copy = pltpu.make_async_copy(w2t_hbm, w2t_v, sems.at[NQ + 6])
    b1_copy = pltpu.make_async_copy(b1_hbm, b1_v, sems.at[NQ + 7])
    b2_copy = pltpu.make_async_copy(b2_hbm, b2_v, sems.at[NQ + 8])

    for c in (wa_copy, x0_copy(0), x0_copy(1), wb_copy, wc_copy, wv_copy,
              x_copy(1), x_copy(2), x_copy(3), wo_copy, w1_copy, b1_copy, b2_copy, w2_copy):
        c.start()

    def x_tile(b, n):
        return xt_v.at[b][:, pl.ds(128 * n, 128)].astype(F32)

    def store_q(b, row, col, q):
        qt_s[pl.ds((b * D + row) // 2, q.shape[0] // 2), pl.ds(col, q.shape[1])] = _pk(
            (q * qscale).astype(BF))

    def store_k(tok, kt):
        pad = jnp.zeros((128 - GW, kt.shape[1]), F32)
        for g in range(NG):
            k = jnp.concatenate([kt[GW * g:GW * (g + 1)], pad], axis=0).T.astype(BF)
            k_s[pl.ds((g * S + tok) // 2, kt.shape[1] // 2), :] = _pk(k)
            if tok == 0:
                kf_s.at[g][...] = k[:VPU_MAX].astype(F32)

    def wt_chunk(lo, n=128):
        wt = wqkv_v[:, pl.ds(lo, n)].astype(F32).T.astype(BF)
        wt_s[pl.ds(lo // 2, n // 2), :] = _pk(wt)
        return wt

    wa_copy.wait()
    x0_copy(0).wait()
    wt3 = wt_chunk(384)
    wt4 = wt_chunk(512)
    xn0 = []
    for n in range(NT):
        if n == 1:
            x0_copy(1).wait()
        d, dm, var = _shifted_moments(x_tile(0, n), 2)
        xn0.append(((d - dm) * lax.rsqrt(var + EPS)).astype(BF))
    xn0 = jnp.concatenate(xn0, axis=1)
    ra = _dot(jnp.concatenate([wt3, wt4], axis=0), xn0[:, :T - 128])
    rb = _dot(wt3, xn0[:, T - 128:])
    wb_copy.wait()
    wc_copy.wait()
    rc = _dot(wt4, xn0[:, T - 128:])
    r34 = jnp.concatenate([ra, jnp.concatenate([rb, rc], axis=0)], axis=1)
    store_q(0, 384, 0, r34[:D - 384])
    store_k(0, jnp.concatenate(
        [r34[D - 384:]] + [_dot(wt_chunk(lo), xn0) for lo in (640, 768)], axis=0))
    for lo in (0, 128):
        store_q(0, lo, 0, _dot(wt_chunk(lo), xn0))
    wt2 = wt_chunk(256)

    wv_copy.wait()
    x_copy(1).wait()
    store_q(0, 256, 0, _dot(wt2, xn0))

    def prep_lhs(dst, top, n):
        zl = jnp.zeros((n, DP - D), F32)
        t = _upk(wt_s[pl.ds(top // 2, n // 2), :]).astype(F32)
        b = _upk(wt_s[pl.ds((top + n) // 2, n // 2), :]).astype(F32)
        ops = _strassen_lhs(t[:, :KH], jnp.concatenate([t[:, KH:], zl], axis=1),
                            b[:, :KH], jnp.concatenate([b[:, KH:], zl], axis=1))
        for k in range(7):
            dst.at[k][...] = _pk(ops[k].astype(BF))

    prep_lhs(aqk_s, 0, D)
    wt_chunk(2 * D, D)
    prep_lhs(av_s, 2 * D, D // 2)

    def rhs_ops(xn):
        zr = jnp.zeros((DP - D, TH), F32)
        ops = _strassen_rhs(xn[:KH, :TH], xn[:KH, TH:],
                            jnp.concatenate([xn[KH:, :TH], zr], axis=0),
                            jnp.concatenate([xn[KH:, TH:], zr], axis=0))
        return [op.astype(BF) for op in ops]

    def ln1_ops(b):
        res = [_layernorm_t(x_tile(b, n)) for n in range(NT)]
        return (rhs_ops(jnp.concatenate([z for z, _ in res], axis=1)),
                [jnp.broadcast_to(r, (8, 128)) for _, r in res])

    def tmp(slot, n):
        return [s_s.at[slot, pl.ds(k * D, n), pl.ds(0, TH)] for k in range(3)]

    def qk_block(b, rhs, deps=None):
        def sink(r, c, z):
            if r == 0:
                store_q(b, 0, c * TH, z)
            else:
                store_k(b * T + c * TH, z)
        _strassen(aqk_s, rhs, tmp(b % 2, D), sink, deps)

    vtail = jnp.where(lax.broadcasted_iota(jnp.int32, (HP - DH, TH), 0) == 0, 1.0, 0.0)

    def v_block(b, rhs, deps=None):
        def sink(r, c, z):
            for i in range(H // 2):
                v = jnp.concatenate([z[DH * i:DH * (i + 1)], vtail], axis=0)
                vp_s[pl.ds(HP // 2 * (r * H // 2 + i), HP // 2),
                     pl.ds(b * T + c * TH, TH)] = _pk(v.astype(BF))
        _strassen(av_s, rhs, tmp(2 + b % 2, D // 2), sink, deps)

    rhs1, r1 = ln1_ops(1)
    qk_block(1, rhs1, {5: r1[0]})
    v_block(0, rhs_ops(xn0.astype(F32)))
    for c in (x_copy(2), x_copy(3), wo_copy, w1_copy, b1_copy):
        c.wait()
    rhs_prev = rhs1
    for b in range(2, NQ):
        rhs, r = ln1_ops(b)
        v_block(b - 1, rhs_prev, {3: r[2], 4: r[3], 7: r[0]})
        qk_block(b, rhs, {5: r[1]})
        rhs_prev = rhs
    v_block(NQ - 1, rhs_prev)

    prow = lax.broadcasted_iota(jnp.int32, (GW // 2, T), 0)
    qzero = jnp.zeros((64 - GW // 2, T), U32)

    def scores_mxu(gi, j, first):
        lo = DH // 2 * j
        q = qt_s[_rows(GW // 2 * gi, GW // 2, 8), :]
        q = jnp.where((prow >= lo) & (prow < lo + DH // 2), q, jnp.uint32(0))
        q = jnp.concatenate([q, qzero], axis=0)
        k = k_s[_rows((gi & (NG - 1)) * (S // 2) + first // 2, (S - first) // 2, 8), :]
        s = _dot(_upk(k), _upk(q))
        s_s.at[j][pl.ds(first, S - first), :] = s
        return s

    def scores_vpu(gi, j, r, dep=None):
        kr = kf_s.at[gi & (NG - 1)][pl.ds(r, 8), :]
        kb = jnp.concatenate([jnp.broadcast_to(kr[:, c:c + 1], (8, T))
                              for c in range(DH * j, DH * (j + 1))], axis=0)
        acc = jnp.sum((kb * qb_s.at[j][...]).reshape(DH, 8, T), axis=0)
        if dep is not None:
            acc = _after(acc, dep)
        s_s.at[j][pl.ds(r, 8), :] = acc
        return acc

    def scores(gi, j):
        s = scores_mxu(gi, j, VPU_KEYS[j])
        nr = s.shape[0] // 8
        early = VPU_KEYS[j] // 8 - VPU_LATE[j]
        skip, frac = VPU_SPAN[j]
        cuts = [math.ceil((u + 1) * (nr * frac - skip) / early + skip) for u in range(early)]
        mx = s[:8]
        for u, (a, b) in enumerate(zip([1] + cuts, cuts + [nr])):
            seg = jnp.concatenate([mx, s[8 * a:8 * b]], axis=0)
            mx = jnp.max(seg.reshape(b - a + 1, 8, T), axis=0)
            if u < early:
                mx = jnp.maximum(mx, scores_vpu(gi, j, 8 * u))
        m_s.at[j][pl.ds(0, 8), :] = mx

    def scores_late(gi, j, o):
        m_s.at[j][pl.ds(8, 8), :] = functools.reduce(jnp.maximum, [
            scores_vpu(gi, j, VPU_KEYS[j] - 8 * (VPU_LATE[j] - u), o[:8, 128 * u:128 * (u + 1)])
            for u in range(VPU_LATE[j])])

    def spread_q(gi, j, pace=None):
        lo = DH * j // 16 * 16
        q = _upk(qt_s[_rows(GW // 2 * gi + lo // 2, 24 if j < GH - 1 else 16, 8), :]).astype(F32)
        for d in range(DH):
            r = DH * j + d - lo
            z = jnp.broadcast_to(q[r:r + 1], (8, T))
            if pace is not None:
                z = _after(z, pace[64 * d:64 * d + 8, :128])
            qb_s.at[j][pl.ds(8 * d, 8), :] = z

    def probs(j, cr=S, lo=0, hi=1):
        m = jnp.max(m_s.at[j][...], axis=0, keepdims=True)
        for c in range(lo, hi):
            p_s.at[j][pl.ds(c * cr // 2, cr // 2), :] = _pk(
                jnp.exp2(s_s.at[j][pl.ds(c * cr, cr), :] - m).astype(BF))

    def pv(gi, j):
        off = (gi & (NG - 1)) * (GH * HP // 2) + j * (HP // 2)
        o = _dot(_upk(vp_s[_rows(off, HP // 2, HP // 2), :]), _upk(p_s.at[j][...]))
        o_s.at[j][...] = o
        return o

    def normalize(gi, j):
        off = gi * (GH * HP // 2) + j * (HP // 2)
        o = o_s.at[j][...]
        o = o * (1.0 / o[DH:DH + 1, :])
        ot_s[_rows(off, HP // 2, HP // 2), :] = _pk(o.astype(BF))

    def prep_wo_w1():
        wtmp_s[pl.ds(0, D // 2), :] = _pk(wo_v[...])
        wtmp_s[pl.ds(D // 2, 8), :] = jnp.zeros((8, D), U32)
        r = lax.broadcasted_iota(jnp.int32, (HP // 2, D), 0)
        wop = jnp.concatenate(
            [jnp.where(r < DH // 2, wtmp_s[pl.ds(DH // 2 * h, HP // 2), :], jnp.uint32(0))
             for h in range(H)], axis=0)
        wot_s[...] = _pk(_upk(wop).astype(F32).T.astype(BF))
        rr = lax.broadcasted_iota(jnp.int32, (DP - D, 128), 0)
        b1 = b1_v[...].astype(F32).reshape(1, F)

        def w1t(r):
            tail = jnp.where(rr == 0, b1[:, 128 * r:128 * (r + 1)], 0.0)
            return jnp.concatenate([w1_v[:, pl.ds(128 * r, 128)].astype(F32), tail], axis=0).T

        for r in range(F // 256):
            t1, t2 = w1t(r), w1t(r + F // 256)
            ops = _strassen_lhs(t1[:, :KH], t1[:, KH:], t2[:, :KH], t2[:, KH:])
            for k in range(7):
                a1_s.at[k][pl.ds(64 * r, 64), :] = _pk(ops[k].astype(BF))

    def prep_w2(c):
        top = w2t_v[_rows(16 * c, 16, 16), :].astype(F32)
        bot = w2t_v[_rows(D // 2 + 16 * c, 16, 16), :].astype(F32)
        ops = _strassen_lhs(top[:, :F // 2], top[:, F // 2:], bot[:, :F // 2], bot[:, F // 2:])
        for k in range(7):
            a2_s.at[k][_rows(8 * c, 8, 8), :] = _pk(ops[k].astype(BF))

    def out_proj(t):
        i, n = t // NT, t % NT
        ot = _upk(ot_s[pl.ds(i * H * HP // 2, H * HP // 2), pl.ds(128 * n, 128)])
        hh = x_tile(i, n) + _dot(_upk(wot_s[...]), ot)
        h_s.at[t][...] = hh
        d = (hh - hh[0:1]).reshape(D // 8, 8, 128)
        raw_s.at[t][pl.ds(0, 8), :] = jnp.sum(d, axis=0)
        raw_s.at[t][pl.ds(8, 8), :] = jnp.sum(d * d, axis=0)

    def ln2_stats(i, dep=None):
        for n in range(NT):
            t = i * NT + n
            s1, s2 = raw_s.at[t][pl.ds(0, 8), :], raw_s.at[t][pl.ds(8, 8), :]
            if dep is not None:
                s1, s2 = _after(s1, dep), _after(s2, dep)
            dm = jnp.sum(s1, axis=0, keepdims=True) * (1.0 / D)
            var = jnp.sum(s2, axis=0, keepdims=True) * (1.0 / D) - dm * dm
            rstd = lax.rsqrt(jnp.maximum(var, 0.0) + EPS)
            st_s.at[t][pl.ds(0, 8), :] = jnp.broadcast_to(h_s.at[t][pl.ds(0, 1), :] + dm, (8, 128))
            st_s.at[t][pl.ds(8, 8), :] = jnp.broadcast_to(rstd, (8, 128))

    htail = jnp.where(lax.broadcasted_iota(jnp.int32, (DP - D, TH), 0) == 0, 1.0, 0.0)

    def hn(i, r, c):
        lo, hi = r * KH, min((r + 1) * KH, D)
        cols = []
        for n in range(NT // 2):
            t = i * NT + c * NT // 2 + n
            z = h_s.at[t][pl.ds(lo, hi - lo), :].reshape((hi - lo) // 8, 8, 128)
            z = (z - st_s.at[t][pl.ds(0, 8), :]) * st_s.at[t][pl.ds(8, 8), :]
            cols.append(z.reshape(hi - lo, 128))
        z = jnp.concatenate(cols, axis=1)
        return z if r == 0 else jnp.concatenate([z, htail], axis=0)

    o_s[...] = jnp.ones(o_s.shape, F32)
    for j in range(GH):
        s = scores_mxu(0, j, 0)
        m_s.at[j][...] = jnp.max(s.reshape(S // 16, 16, T), axis=0)
        spread_q(1, j, s)
        if j == 0:
            prep_wo_w1()
    w2_copy.wait()

    def body(gi, carry):
        for j in range(GH):
            normalize(jnp.maximum(gi - 1, 0), j)
            probs(j)
            scores(gi + 1, j)
            scores_late(gi + 1, j, pv(gi, j))
            spread_q(jnp.minimum(gi + 2, NGI - 1), j)
        prep_w2(jnp.minimum(gi, D // 32 - 1))
        return carry

    lax.fori_loop(0, NGI - 1, body, 0)

    gl = NGI - 1
    nfirst = (NQ - 1) * NT - 2
    nch = S // 16
    for j in range(GH):
        normalize(gl - 1, j)
    for t in range(nfirst):
        lo, hi = t * GH * nch // nfirst, (t + 1) * GH * nch // nfirst
        while lo < hi:
            j = lo // nch
            e = min(hi, (j + 1) * nch)
            probs(j, 16, lo - j * nch, e - j * nch)
            lo = e
        out_proj(t)
    b2_copy.wait()
    b2_s[...] = jnp.broadcast_to(b2_v[...].astype(F32).reshape(1, D), (128, D)).T
    for j in range(GH):
        pv(gl, j)
        normalize(gl, j)
    ln2_stats(0)
    first_s[...] = _pk(hn(0, 1, 1).astype(BF))
    for t in range(nfirst, NQ * NT):
        out_proj(t)

    def out_copy(i, r, t):
        return pltpu.make_async_copy(
            out_v.at[(i * 2 + r) * NT + t],
            out_hbm.at[pl.ds(r * D // 2, D // 2), _rows(i * T + t * 128, 128, 128)], osem)

    tmps = [s_s.at[k // 2, pl.ds(0, F // 2), pl.ds(k % 2 * TH, TH)] for k in range(6)]
    ab = [p_s.at[k // 2, pl.ds(0, F // 4), pl.ds(k % 2 * TH, TH)] for k in range(7)]

    def ffn(i, carry):
        a11, a12, a21 = tmps[3:]

        def put(k, val):
            ab[k - 1][...] = _pk(val.astype(BF))

        def sink(r, c, z):
            a = jnp.square(jnp.maximum(z, 0.0))
            if (r, c) == (0, 1):
                a12[...] = a
            elif (r, c) == (1, 0):
                a21[...] = a
            elif (r, c) == (0, 0):
                a11[...] = a
                put(2, a)
                put(4, a21[...] - a)
                put(6, a + a12[...])
            else:
                put(1, a11[...] + a)
                put(3, a12[...] - a)
                put(5, a)
                put(7, a21[...] + a)

        rhs = [op.astype(BF) for op in _strassen_rhs(
            hn(i, 0, 0), hn(i, 0, 1), hn(i, 1, 0), hn(i, 1, 1))]
        rhs[4] = _upk(first_s[...])
        _strassen(a1_s, rhs, tmps[:3], sink)

        def emit(r, c, y):
            rows = pl.ds(r * D // 2, D // 2)
            for n in range(NT // 2):
                t = c * NT // 2 + n
                z = h_s.at[i * NT + t][rows, :] + b2_s[rows, :] + y[:, 128 * n:128 * (n + 1)]
                out_v.at[(i * 2 + r) * NT + t][...] = z.astype(BF)
                out_copy(i, r, t).start()

        m = lambda k: _dot(_upk(a2_s.at[k - 1][...]), _upk(ab[k - 1][...]))
        m2, m4 = m(2), m(4)
        nxt = jnp.minimum(i + 1, NQ - 1)
        ln2_stats(nxt, m2[:8, :128])
        first_s[...] = _pk(hn(nxt, 1, 1).astype(BF))
        emit(1, 0, m2 + m4)
        m6, m1, m3 = m(6), m(1), m(3)
        emit(1, 1, m1 - m2 + m3 + m6)
        m5 = m(5)
        emit(0, 1, m3 + m5)
        m7 = m(7)
        emit(0, 0, m1 + m4 - m5 + m7)
        return carry

    lax.fori_loop(0, NQ, ffn, 0)
    for i in range(NQ):
        for r in range(2):
            for t in range(NT):
                out_copy(i, r, t).wait()


@jax.jit
def pallas_sequential_preLN__mha_block__dense_activation_squared_relu__prompt_kernel(
    A_x: jax.Array,
    A_wqkv: jax.Array,
    A_wo: jax.Array,
    B_x: jax.Array,
    B_w1: jax.Array,
    B_b1: jax.Array,
    B_w2: jax.Array,
    B_b2: jax.Array,
):
    B, S, D = A_x.shape
    F = B_w1.shape[1]
    T = 512
    NQ = S // T
    assert B == 1 and D == H * DH and NQ == 4 and F % 256 == 0
    xt = jnp.swapaxes(A_x, 1, 2).reshape(D, S)
    hbm = pl.BlockSpec(memory_space=pltpu.MemorySpace.HBM)
    out = pl.pallas_call(
        functools.partial(_kernel, S=S, D=D, F=F, T=T),
        in_specs=[hbm] * 7,
        out_specs=hbm,
        out_shape=jax.ShapeDtypeStruct((D, S), A_x.dtype),
        scratch_shapes=[
            pltpu.VMEM((NQ, D, T), BF),
            pltpu.VMEM((D, 3 * D), BF),
            pltpu.VMEM((D, D), BF),
            pltpu.VMEM((D, F), BF),
            pltpu.VMEM((D, F), BF),
            pltpu.VMEM((S // 64, D // 2, 128), BF),
            pltpu.SemaphoreType.DMA((NQ + 10,)),
            pltpu.SemaphoreType.DMA(()),
            pltpu.VMEM((3 * D // 2, D), U32),
            pltpu.VMEM((7, D // 2, DP // 2), U32),
            pltpu.VMEM((7, D // 4, DP // 2), U32),
            pltpu.VMEM((D // 2, H * HP), U32),
            pltpu.VMEM((7, F // 4, DP // 2), U32),
            pltpu.VMEM((8, D // 4, F // 2), U32),
            pltpu.VMEM((D, 128), F32),
            pltpu.VMEM((D // 2 + 8, D), U32),
            pltpu.VMEM((NG * S // 2, 128), U32),
            pltpu.VMEM((NQ * D // 2, T), U32),
            pltpu.VMEM((H * HP // 2, S), U32),
            pltpu.VMEM((NQ * H * HP // 2, T), U32),
            pltpu.VMEM((S // 128, D, 128), F32),
            pltpu.VMEM((S // 128, 16, 128), F32),
            pltpu.VMEM((S // 128, 16, 128), F32),
            pltpu.VMEM((DP // 4, T // 2), U32),
            pltpu.VMEM((GH, DH * 8, T), F32),
            pltpu.VMEM((NG, VPU_MAX, 128), F32),
            pltpu.VMEM((GH, S, T), F32),
            pltpu.VMEM((GH, S // 2, T), U32),
            pltpu.VMEM((GH, 16, T), F32),
            pltpu.VMEM((GH, HP, T), F32),
            pltpu.VMEM((F,), BF),
            pltpu.VMEM((D,), BF),
        ],
        compiler_params=pltpu.CompilerParams(vmem_limit_bytes=100 * 1024 * 1024,
                                             disable_bounds_checks=True,
                                             disable_semaphore_checks=True),
    )(xt, A_wqkv, A_wo, B_w1, B_b1, B_w2.T, B_b2)
    return jnp.swapaxes(out.reshape(B, D, S), 1, 2)
```
